```python
import jax
import jax.numpy as jnp

def _softmax(x, axis=-1):
    return jax.nn.softmax(x, axis=axis)
def _gelu(x):
    return jax.nn.gelu(x, approximate=True)
def _silu(x):
    return jax.nn.silu(x)
def _sigmoid(x):
    return jax.nn.sigmoid(x)
def _layernorm(x, axis=-1, eps=1e-5):
    m = jnp.mean(x, axis=axis, keepdims=True)
    v = jnp.var(x, axis=axis, keepdims=True)
    return (x - m) / jnp.sqrt(v + eps)
def _scatter_add(tgt, idx, src, axis=0):
    return tgt.at[idx].add(src)
def _segment_sum(src, seg, n):
    return jax.ops.segment_sum(src, seg, n)
class _Rng:
    def __init__(self, key):
        self._k = key
    def _next(self):
        self._k, sub = jax.random.split(self._k)
        return sub
    def normal(self, shape):
        return jax.random.normal(self._next(), shape, dtype=jnp.bfloat16)
    def randint(self, lo, hi, shape):
        return jax.random.randint(self._next(), shape, lo, hi, dtype=jnp.int32)
    def uniform(self, shape, lo=0.0, hi=1.0):
        return jax.random.uniform(self._next(), shape, jnp.bfloat16, lo, hi)
    def permutation(self, n):
        return jax.random.permutation(self._next(), n)


kernel_name = 'recurrent_scan__sliding_block_cached__moe_arch_mod__prompt'

def setup_inputs():
    _rng = _Rng(jax.random.key(int.from_bytes(__import__("os").urandom(4), "little")))
    _w = (lambda a: (lambda t: t.astype(jnp.bfloat16) if jnp.issubdtype(t.dtype, jnp.floating) else t)(jnp.asarray(a)))
    def _A_setup():
        B, Sq, D = 1, 2048, 640
        Hq, Hkv, Sk, Dh = 32, 32, 2048, 192
        assert Hq % Hkv == 0, (Hq, Hkv)
        return {
            "x": _w((lambda *s: _rng.normal(s) * 0.05)(B, Sq, D)),
            "k_cache": _w((lambda *s: _rng.normal(s) * 0.05)(B, Hkv, Sk, Dh)),
            "v_cache": _w((lambda *s: _rng.normal(s) * 0.05)(B, Hkv, Sk, Dh)),
            "wq": _w((lambda *s: _rng.normal(s) * 0.05)(D, Hq * Dh) * (D ** -0.5)),
            "wo": _w((lambda *s: _rng.normal(s) * 0.05)(Hq * Dh, D) * ((Hq * Dh) ** -0.5)),
        }
    _A_in = _A_setup()

    def _B_setup():
        B, S, D, F, C = 1, 2048, 640, 1536, 2
        return {
            "x": _w((lambda *s: _rng.normal(s) * 0.05)(B, S, D)),
            "w_r": _w((lambda *s: _rng.normal(s) * 0.05)(D)),
            "w_gate": _w((lambda *s: _rng.normal(s) * 0.05)(D, F)),
            "w_up": _w((lambda *s: _rng.normal(s) * 0.05)(D, F)),
            "w_down": _w((lambda *s: _rng.normal(s) * 0.05)(F, D)),
        }
    _B_in = _B_setup()

    return {
        "A_x": _A_in["x"],
        "A_k_cache": _A_in["k_cache"],
        "A_v_cache": _A_in["v_cache"],
        "A_wq": _A_in["wq"],
        "A_wo": _A_in["wo"],
        "B_x": _B_in["x"],
        "B_w_r": _B_in["w_r"],
        "B_w_gate": _B_in["w_gate"],
        "B_w_up": _B_in["w_up"],
        "B_w_down": _B_in["w_down"],
    }

def reference(A_x, A_k_cache, A_v_cache, A_wq, A_wo, B_x, B_w_r, B_w_gate, B_w_up, B_w_down):
    def _A_ref(x, k_cache, v_cache, wq, wo):
        B, Sq, D = x.shape
        Hq, Dh = 32, 192
        Hkv, Sk = k_cache.shape[1], k_cache.shape[2]
        W = min(4096, max(256, Sk // 4))
        rep = Hq // Hkv
        q = (lambda x, *d: x.transpose(*d))((x @ wq).reshape(B, Sq, Hq, Dh), 0, 2, 1, 3)
        k = jnp.repeat(k_cache[:, :, Sk - W:, :], rep, axis=1)
        v = jnp.repeat(v_cache[:, :, Sk - W:, :], rep, axis=1)
        scores = jnp.einsum("bhqd,bhkd->bhqk", q, k) * (Dh ** -0.5)
        p = _softmax(scores, axis=-1)
        o = jnp.einsum("bhqk,bhkd->bhqd", p, v)
        return (lambda x, *d: x.transpose(*d))(o, 0, 2, 1, 3).reshape(B, Sq, Hq * Dh) @ wo

    def _B_ref(x, w_r, w_gate, w_up, w_down):
        B, S, D = x.shape
        C = 2
        r = x @ w_r
        idx = jnp.argsort(-r, axis=-1)[:, :C]
        idx_e = jnp.repeat(idx.reshape(B, C, 1), D, axis=2)
        x_sel = jnp.take_along_axis(x, idx_e, axis=1)
        g = _silu(x_sel @ w_gate)
        u = x_sel @ w_up
        y = (g * u) @ w_down
        r_sel = _sigmoid(jnp.take_along_axis(r, idx, axis=1))
        y = y * r_sel.reshape(B, C, 1)
        b_off = (jnp.arange(B) * S).reshape(B, 1)
        flat_idx = (idx + b_off).reshape(B * C)
        zero = (x * 0.0).reshape(B * S, D)
        upd = _scatter_add(zero, flat_idx, y.reshape(B * C, D), axis=0)
        return x + upd.reshape(B, S, D)

    x = A_x
    xn = _layernorm(x, axis=-1)
    s = _A_ref(xn, A_k_cache, A_v_cache, A_wq, A_wo)
    g = _silu(_B_ref(xn, B_w_r, B_w_gate, B_w_up, B_w_down))
    return x + s * g
```

```python
import contextlib
import functools
import math

import jax
import jax.numpy as jnp
from jax import lax
import jax.experimental.pallas as pl
import jax.experimental.pallas.tpu as pltpu

F32 = jnp.float32
BF16 = jnp.bfloat16
LANE = 128
SUB = 8


def _nt(a, b):
    return lax.dot_general(a, b, (((1,), (1,)), ((), ())), preferred_element_type=F32)


def _nn(a, b):
    return jnp.dot(a, b, preferred_element_type=F32)


def _nn_q(a, b):
    return jnp.dot(a, b, preferred_element_type=F32)


def _nn_pv(a, b):
    return jnp.dot(a, b, preferred_element_type=F32)


def _nn_wo(a, b):
    return jnp.dot(a, b, preferred_element_type=F32)


def _silu(x):
    h = 0.5 * x
    return h + h * jnp.tanh(h)


def _kernel(x_hbm, kt_hbm, vt_hbm, wq_hbm, wo_hbm, wr_ref, wg_hbm, wu_hbm, wd_hbm,
            out_hbm,
            x_buf, xn_ref, acc_ref, out_buf, wq_buf, wo_buf, kt_buf, vt_buf, kp_ref,
            q_st, ot_st, s0_ref, s1_ref, top_ref, y_ref, idx_ref, wg_ref, wu_ref, wd_ref,
            sem_x, sem_wq, sem_wo, sem_k, sem_v, sem_f, sem_o,
            *, TQ, NP, DH, W, eps, scopes, only):
    S, D = x_buf.shape
    U = S // TQ
    HALF = U // 2
    PW = 2 * DH
    PADW = 2 * LANE
    SK = kt_hbm.shape[-1]
    c = (DH ** -0.5) * math.log2(math.e)
    step = pl.program_id(0)
    z = step // (NP + 1)
    s_refs = (s0_ref, s1_ref)

    def scope(name):
        return jax.named_scope(name) if scopes else contextlib.nullcontext()

    def cp_x(t):
        return pltpu.make_async_copy(x_hbm.at[pl.ds(t * TQ, TQ)], x_buf.at[pl.ds(t * TQ, TQ)], sem_x.at[t])

    def src(p):
        return min(p, NP - 1) if isinstance(p, int) else jnp.minimum(p, NP - 1)

    def col(p):
        return p * PW if isinstance(p, int) else pl.multiple_of(p * PW, LANE)

    def cp_wq(p, slot):
        return pltpu.make_async_copy(wq_hbm.at[:, pl.ds(col(src(p)), PW)], wq_buf.at[slot], sem_wq.at[slot])

    def cp_wo(p, slot):
        return pltpu.make_async_copy(wo_hbm.at[pl.ds(col(src(p)), PW)], wo_buf.at[slot], sem_wo.at[slot])

    def cp_k(p, slot):
        return pltpu.make_async_copy(kt_hbm.at[0, pl.ds(2 * src(p), 2), :, pl.ds(SK - W, W)], kt_buf.at[slot], sem_k.at[slot])

    def cp_v(p, slot):
        return pltpu.make_async_copy(vt_hbm.at[0, pl.ds(2 * src(p), 2), :, pl.ds(SK - W, W)], vt_buf.at[slot], sem_v.at[slot])

    def cp_ffn():
        return (pltpu.make_async_copy(wg_hbm, wg_ref, sem_f.at[0]),
                pltpu.make_async_copy(wu_hbm, wu_ref, sem_f.at[1]),
                pltpu.make_async_copy(wd_hbm, wd_ref, sem_f.at[2]))

    def cp_out(t):
        return pltpu.make_async_copy(out_buf.at[pl.ds(t * TQ, TQ)], out_hbm.at[pl.ds(t * TQ, TQ)], sem_o.at[t])

    def rows(u, part=0, nparts=1):
        n = TQ // nparts
        return pl.ds(u * TQ + part * n, n)

    def layernorm(u, top):
        r = rows(u)
        x = x_buf[r, :].astype(F32)
        m = jnp.mean(x, axis=-1, keepdims=True)
        xc = x - m
        v = jnp.mean(xc * xc, axis=-1, keepdims=True)
        xn = (xc * lax.rsqrt(v + eps)).astype(BF16)
        xn_ref[r, :] = xn
        acc_ref[r, :] = jnp.zeros((TQ, D), F32)
        sc = jnp.sum(xn.astype(F32) * wr_ref[...].astype(F32), axis=-1, keepdims=True)
        sc = jnp.broadcast_to(sc.astype(BF16).astype(F32), (TQ, LANE))
        sub = lax.broadcasted_iota(jnp.int32, (SUB, LANE), 0)
        for t in range(TQ // SUB):
            val = sc[t * SUB:(t + 1) * SUB]
            idx = sub + (u * TQ + t * SUB)
            if top is None:
                top = (val, idx, jnp.full((SUB, LANE), -jnp.inf, F32), idx)
                continue
            m1, i1, m2, i2 = top
            g1 = val > m1
            g2 = val > m2
            top = (jnp.where(g1, val, m1), jnp.where(g1, idx, i1),
                   jnp.where(g1, m1, jnp.where(g2, val, m2)),
                   jnp.where(g1, i1, jnp.where(g2, idx, i2)))
        return top

    def prep_k(src_slot, dst_slot):
        zz = jnp.zeros((PADW - DH, W), BF16)
        kp_ref[dst_slot, 0] = jnp.concatenate([kt_buf[src_slot, 0], zz], axis=0).T
        kp_ref[dst_slot, 1] = jnp.concatenate([zz, kt_buf[src_slot, 1]], axis=0).T

    def qproj_tile(u, n, slot):
        w = wq_buf[slot, :, n * LANE:(n + 1) * LANE]
        return (_nn_q(xn_ref[rows(u), :], w) * c).astype(BF16)

    def qproj_split(u, slot):
        parts = [(_nn_q(xn_ref[rows(u, t, 4), :], wq_buf[slot]) * c).astype(BF16) for t in range(4)]
        q = jnp.concatenate(parts, axis=0)
        return [q[:, n * LANE:(n + 1) * LANE] for n in range(3)]

    def qk(q, h, slot):
        st = _nt(kp_ref[slot, h], jnp.concatenate(q[h:h + 2], axis=1))
        s_refs[h][0] = st
        return jnp.max(st, axis=0, keepdims=True)

    def softmax(m, h):
        e = jnp.exp2(s_refs[h][z] - m)
        return e.astype(BF16), jnp.sum(e, axis=0, keepdims=True)

    def pv(p, l, h, slot):
        return (_nn_pv(vt_buf[slot, h], p) * (1.0 / l)).astype(BF16)

    def finish(u, val, n0, n1, part, nparts):
        n = TQ // nparts
        r = rows(u, part, nparts)
        cs = slice(n0 * LANE, n1 * LANE)
        rid = u * TQ + part * n + lax.broadcasted_iota(jnp.int32, (n, 1), 0)
        upd = (jnp.where(rid == idx_ref[0], y_ref[0:1, cs], 0.0)
               + jnp.where(rid == idx_ref[1], y_ref[1:2, cs], 0.0))
        g = _silu(xn_ref[r, cs].astype(F32) + upd)
        out_buf[r, cs] = (x_buf[r, cs].astype(F32) + val * g).astype(out_buf.dtype)

    def wo_cols(u, o, slot, n0, n1, part=0, nparts=1, final=False):
        n = TQ // nparts
        r = rows(u, part, nparts)
        cs = slice(n0 * LANE, n1 * LANE)
        val = acc_ref[r, cs] + _nn_wo(o[part * n:(part + 1) * n], wo_buf[slot, :, cs])
        if final:
            finish(u, val, n0, n1, part, nparts)
        else:
            acc_ref[r, cs] = val

    def unit(q, prev, bslot, a, cc, final=False, mid=None):
        m0 = qk(q, 0, bslot)
        m1 = qk(q, 1, bslot)
        if mid is not None:
            mid()
        p0 = softmax(m0, 0)
        p1 = softmax(m1, 1)
        if cc is not None:
            o = prev.T
        if a is not None and cc is not None:
            qn = []
            for n in range(3):
                qn.append(qproj_tile(a[0], n, a[1]))
                wo_cols(cc[0], o, cc[1], n, n + 1, final=final)
            wo_cols(cc[0], o, cc[1], 3, 5, 0, 2, final=final)
            wo_cols(cc[0], o, cc[1], 3, 5, 1, 2, final=final)
        elif a is not None:
            qn = qproj_split(a[0], a[1])
        else:
            qn = None
            for t in range(4):
                wo_cols(cc[0], o, cc[1], 0, 5, t, 4, final=final)
        o0 = pv(*p0, 0, bslot)
        o1 = pv(*p1, 1, bslot)
        return qn, jnp.concatenate([o0, o1], axis=0)

    def load_carry():
        qv = q_st[...]
        return [qv[:, n * LANE:(n + 1) * LANE] for n in range(3)], ot_st[...]

    def store_carry(q, prev):
        q_st[...] = jnp.concatenate(q, axis=1)
        ot_st[...] = prev

    def prologue():
        cp_x(0).start()
        cp_wq(0, 0).start()
        cp_k(0, 0).start()
        cp_x(1).start()
        cp_v(0, 0).start()
        cp_x(0).wait()
        top = layernorm(0, None)
        for t in range(2, U):
            cp_x(t).start()
            if t == 3:
                cp_wo(0, 0).start()
        cp_k(1, 1).start()
        cp_wq(1, 1).start()
        cp_v(1, 1).start()
        cp_wo(1, 1).start()
        for cp in cp_ffn():
            cp.start()
        cp_wq(0, 0).wait()
        cp_k(0, 0).wait()
        cp_x(1).wait()
        q = qproj_split(0, 0)
        prep_k(0, 0)
        top = layernorm(1, top)
        cp_v(0, 0).wait()
        prev = None
        nxt = 2
        for u in range(HALF):
            if u == 1:
                cp_x(2).wait()
                cp_x(3).wait()
                cp_wo(0, 0).wait()
            if u == 2:
                cp_k(2, 0).start()
                for t in range(4, U):
                    cp_x(t).wait()
                cp_k(1, 1).wait()
            if u >= 1:
                for _ in range(2):
                    if nxt < U:
                        top = layernorm(nxt, top)
                        nxt += 1
            q, prev = unit(q, prev, 0, (u + 1, 0), (u - 1, 0) if u > 0 else None,
                           mid=(lambda: prep_k(1, 1)) if u == HALF - 1 else None)
        assert nxt == U
        store_carry(q, prev)
        top_ref[0] = top[0]
        top_ref[1] = top[2]
        top_ref[2] = top[1].astype(F32)
        top_ref[3] = top[3].astype(F32)

    def ffn_block():
        for cp in cp_ffn():
            cp.wait()
        vals = jnp.concatenate([top_ref[0], top_ref[1]], axis=0)
        ids = jnp.concatenate([top_ref[2], top_ref[3]], axis=0)
        big = float(S)
        m1 = jnp.max(vals)
        f1 = jnp.min(jnp.where(vals == m1, ids, big))
        vals2 = jnp.where(ids == f1, -jnp.inf, vals)
        m2 = jnp.max(vals2)
        f2 = jnp.min(jnp.where(jnp.logical_and(vals2 == m2, ids != f1), ids, big))
        i1 = jnp.minimum(f1.astype(jnp.int32), S - 1)
        i2 = jnp.minimum(f2.astype(jnp.int32), S - 1)
        idx_ref[0] = i1
        idx_ref[1] = i2
        sub = lax.broadcasted_iota(jnp.int32, (16, D), 0)

        def pick(ix):
            base = pl.multiple_of((ix // 16) * 16, 16)
            blk = xn_ref[pl.ds(base, 16), :].astype(F32)
            return jnp.sum(jnp.where(sub == ix - base, blk, 0.0), axis=0, keepdims=True)

        xs = jnp.where(sub == 0, pick(i1), jnp.where(sub == 1, pick(i2), 0.0)).astype(BF16)
        gg = _nn(xs, wg_ref[...])
        uu = _nn(xs, wu_ref[...])
        hmid = (_silu(gg) * uu).astype(BF16)
        y = _nn(hmid, wd_ref[...])
        rs = jnp.where(sub == 0, m1, m2)
        y_ref[...] = y * jax.nn.sigmoid(rs)

    def main(j):
        s0 = j % 3
        s1 = jnp.where(s0 == 2, 0, s0 + 1)
        s2 = jnp.where(s0 == 0, 2, s0 - 1)
        k0 = j & 1
        k1 = 1 - k0
        cp_wq(j + 2, s2).start()
        cp_v(j + 2, s2).start()
        cp_wo(j + 2, s2).start()
        cp_k(j + 3, k1).start()
        cp_wq(j + 1, s1).wait()
        cp_k(j + 2, k0).wait()
        cp_v(j + 1, s1).wait()
        cp_wo(j + 1, s1).wait()
        q, prev = load_carry()
        for v in range(U):
            u = (HALF + v) % U
            bs = s1 if v >= U - HALF else s0
            as_ = s1 if v + 1 >= U - HALF else s0
            cs_ = s1 if v - 1 >= U - HALF else s0
            mid = (lambda: prep_k(k0, s2)) if v == U - 1 else None
            q, prev = unit(q, prev, bs, ((u + 1) % U, as_), ((u - 1) % U, cs_), mid=mid)
        store_carry(q, prev)

    def tail():
        p = NP - 1
        cp_wq(p + 1, (p + 1) % 3).wait()
        cp_k(p + 2, (p + 2) % 2).wait()
        cp_v(p + 1, (p + 1) % 3).wait()
        cp_wo(p + 1, (p + 1) % 3).wait()
        q, prev = load_carry()
        for u in range(HALF - 1):
            finish(u, acc_ref[rows(u), :], 0, D // LANE, 0, 1)
            cp_out(u).start()
        for u in range(HALF, U):
            a = (u + 1, p % 3) if u + 1 < U else None
            q, prev = unit(q, prev, p % 3, a, (u - 1, p % 3), final=True)
            cp_out(u - 1).start()
        o = prev.T
        for t in range(4):
            wo_cols(U - 1, o, p % 3, 0, 5, t, 4, final=True)
        cp_out(U - 1).start()
        for t in range(U):
            cp_out(t).wait()

    if "P" in only:
        @pl.when(step == 0)
        def _():
            with scope("P"):
                prologue()

    if "F" in only:
        @pl.when(step == 2)
        def _():
            with scope("ffn"):
                ffn_block()

    if "M" in only:
        @pl.when(jnp.logical_and(step > 0, step < NP))
        def _():
            with scope("M"):
                main(step - 1)

    if "T" in only:
        @pl.when(step == NP)
        def _():
            with scope("T"):
                tail()


def _build(TQ=256, VMEM_MB=100, scopes=False, only="PFMT"):
    def fn(A_x, A_k_cache, A_v_cache, A_wq, A_wo, B_x, B_w_r, B_w_gate, B_w_up, B_w_down):
        B, S, D = A_x.shape
        _, H, SK, DH = A_k_cache.shape
        W = min(4096, max(256, SK // 4))
        assert B == 1 and H % 2 == 0
        NP = H // 2
        U = S // TQ
        FF = B_w_gate.shape[1]
        x = A_x.reshape(S, D)
        wr = B_w_r.reshape(1, D)
        kern = functools.partial(_kernel, TQ=TQ, NP=NP, DH=DH, W=W, eps=1e-5, scopes=scopes, only=only)
        hbm = pl.BlockSpec(memory_space=pl.ANY)
        out = pl.pallas_call(
            kern,
            grid=(NP + 1,),
            in_specs=[hbm, hbm, hbm, hbm, hbm,
                      pl.BlockSpec((1, D), lambda j: (0, 0)),
                      hbm, hbm, hbm],
            out_specs=hbm,
            out_shape=jax.ShapeDtypeStruct((S, D), A_x.dtype),
            scratch_shapes=[
                pltpu.VMEM((S, D), BF16),
                pltpu.VMEM((S, D), BF16),
                pltpu.VMEM((S, D), F32),
                pltpu.VMEM((S, D), A_x.dtype),
                pltpu.VMEM((3, D, 2 * DH), BF16),
                pltpu.VMEM((3, 2 * DH, D), BF16),
                pltpu.VMEM((2, 2, DH, W), BF16),
                pltpu.VMEM((3, 2, DH, W), BF16),
                pltpu.VMEM((3, 2, W, 2 * LANE), BF16),
                pltpu.VMEM((TQ, 2 * DH), BF16),
                pltpu.VMEM((2 * DH, TQ), BF16),
                pltpu.VMEM((1, W, TQ), F32),
                pltpu.VMEM((1, W, TQ), F32),
                pltpu.VMEM((4, SUB, LANE), F32),
                pltpu.VMEM((16, D), F32),
                pltpu.SMEM((2,), jnp.int32),
                pltpu.VMEM((D, FF), BF16),
                pltpu.VMEM((D, FF), BF16),
                pltpu.VMEM((FF, D), BF16),
                pltpu.SemaphoreType.DMA((U,)),
                pltpu.SemaphoreType.DMA((3,)),
                pltpu.SemaphoreType.DMA((3,)),
                pltpu.SemaphoreType.DMA((2,)),
                pltpu.SemaphoreType.DMA((3,)),
                pltpu.SemaphoreType.DMA((3,)),
                pltpu.SemaphoreType.DMA((U,)),
            ],
            compiler_params=pltpu.CompilerParams(
                dimension_semantics=("arbitrary",),
                vmem_limit_bytes=VMEM_MB * 1024 * 1024),
            name="fused_attn_moe",
        )(x, jnp.swapaxes(A_k_cache, 2, 3), jnp.swapaxes(A_v_cache, 2, 3), A_wq, A_wo, wr,
          B_w_gate, B_w_up, B_w_down)
        return out.reshape(B, S, D)
    return fn


@jax.jit
def pallas_recurrent_scan__sliding_block_cached__moe_arch_mod__prompt_kernel(
        A_x, A_k_cache, A_v_cache, A_wq, A_wo, B_x, B_w_r, B_w_gate, B_w_up, B_w_down):
    return _build()(A_x, A_k_cache, A_v_cache, A_wq, A_wo, B_x, B_w_r, B_w_gate, B_w_up, B_w_down)
```

```python
import contextlib
import functools
import math

import jax
import jax.numpy as jnp
from jax import lax
import jax.experimental.pallas as pl
import jax.experimental.pallas.tpu as pltpu

F32 = jnp.float32
BF16 = jnp.bfloat16
LANE = 128
SUB = 8
NSLOT = 4


def _nt(a, b):
    return lax.dot_general(a, b, (((1,), (1,)), ((), ())), preferred_element_type=F32)


def _nn(a, b):
    return jnp.dot(a, b, preferred_element_type=F32)


def _nn_q(a, b):
    return jnp.dot(a, b, preferred_element_type=F32)


def _nn_pv(a, b):
    return jnp.dot(a, b, preferred_element_type=F32)


def _nn_wo(a, b):
    return jnp.dot(a, b, preferred_element_type=F32)


def _silu(x):
    h = 0.5 * x
    return h + h * jnp.tanh(h)


def _kernel(x_hbm, kt_hbm, vt_hbm, wq_hbm, wo_hbm, wr_hbm, wg_hbm, wu_hbm, wd_hbm,
            out_hbm,
            x_buf, xn_ref, xg_ref, acc_ref, out_buf, wq_buf, wo_buf, kt_buf, vt_buf, kp_ref,
            q_st, ot_st, s0_ref, s1_ref, xs_ref, rs_ref, idx_ref, wr_ref, wg_ref, wu_ref, wd_ref,
            sem_x, sem_wq, sem_wo, sem_k, sem_v, sem_f, sem_o,
            *, TQ, NP, DH, W, eps, scopes, only, R, G, RF32, GT, ESTART, FENCE):
    S, D = x_buf.shape
    U = S // TQ
    PW = 2 * DH
    PADW = 2 * LANE
    SK = kt_hbm.shape[-1]
    c = (DH ** -0.5) * math.log2(math.e)
    step = pl.program_id(0)
    z = step // (NP + 1)
    s_refs = (s0_ref, s1_ref)

    def scope(name):
        return jax.named_scope(name) if scopes else contextlib.nullcontext()

    def slot_of(p):
        return p % NSLOT if isinstance(p, int) else p & (NSLOT - 1)

    def cp_x(t):
        return pltpu.make_async_copy(x_hbm.at[pl.ds(t * TQ, TQ)], x_buf.at[pl.ds(t * TQ, TQ)], sem_x.at[t])

    def col(p):
        return p * PW if isinstance(p, int) else pl.multiple_of(p * PW, LANE)

    def cp_wq(p):
        s = slot_of(p)
        return pltpu.make_async_copy(wq_hbm.at[:, pl.ds(col(p), PW)], wq_buf.at[s], sem_wq.at[s])

    def cp_wo(p):
        s = slot_of(p)
        return pltpu.make_async_copy(wo_hbm.at[pl.ds(col(p), PW)], wo_buf.at[s], sem_wo.at[s])

    def cp_k(p):
        s = slot_of(p)
        return pltpu.make_async_copy(kt_hbm.at[0, pl.ds(2 * p, 2), :, pl.ds(SK - W, W)], kt_buf.at[s], sem_k.at[s])

    def cp_v(p):
        s = slot_of(p)
        return pltpu.make_async_copy(vt_hbm.at[0, pl.ds(2 * p, 2), :, pl.ds(SK - W, W)], vt_buf.at[s], sem_v.at[s])

    def cp_pair(p):
        return (cp_wq(p), cp_v(p), cp_wo(p))

    def cp_ffn():
        return (pltpu.make_async_copy(wg_hbm, wg_ref, sem_f.at[0]),
                pltpu.make_async_copy(wu_hbm, wu_ref, sem_f.at[1]),
                pltpu.make_async_copy(wd_hbm, wd_ref, sem_f.at[2]))

    def cp_out(t, part=0, nparts=1):
        r = rows(t, part, nparts)
        return pltpu.make_async_copy(out_buf.at[r], out_hbm.at[r], sem_o.at[t + part])

    def rows(u, part=0, nparts=1):
        n = TQ // nparts
        return pl.ds(u * TQ + part * n, n)

    def tie(v, const):
        cb = lax.bitcast_convert_type(jnp.float32(const), jnp.int32)
        vb = lax.bitcast_convert_type(v, jnp.int32)
        return lax.bitcast_convert_type(jnp.minimum((vb & 0x7FFFFFFF) | cb, cb), F32)

    def layernorm(u, top, chain=None):
        GR = 16
        wr = wr_ref[...].astype(F32).reshape(1, D)
        sub = lax.broadcasted_iota(jnp.int32, (SUB, LANE), 0)
        acc_ref[rows(u), :] = jnp.zeros((TQ, D), F32)
        for t in range(TQ // GR):
            r = pl.ds(u * TQ + t * GR, GR)
            x = x_buf[r, :].astype(F32)
            ssum = jnp.sum(x, axis=-1, keepdims=True)
            if chain is not None and len(chain) >= G:
                m = ssum * tie(chain[-G], 1.0 / D)
            else:
                m = ssum * (1.0 / D)
            xc = x - m
            v = jnp.sum(xc * xc, axis=-1, keepdims=True) * (1.0 / D)
            xf = xc * lax.rsqrt(v + eps)
            xn = xf.astype(BF16)
            xn_ref[r, :] = xn
            xg_ref[r, :] = xn
            sc = jnp.sum((xf if RF32 else xn.astype(F32)) * wr, axis=-1, keepdims=True)
            sc = sc.astype(BF16).astype(F32)
            if chain is not None:
                chain.append(sc)
            scb = jnp.broadcast_to(sc, (GR, LANE))
            for h in range(GR // SUB):
                val = scb[h * SUB:(h + 1) * SUB]
                idx = sub + (u * TQ + t * GR + h * SUB)
                if top is None:
                    top = (val, idx, jnp.full((SUB, LANE), -jnp.inf, F32), idx)
                    continue
                m1, i1, m2, i2 = top
                g1 = val > m1
                g2 = val > m2
                top = (jnp.where(g1, val, m1), jnp.where(g1, idx, i1),
                       jnp.where(g1, m1, jnp.where(g2, val, m2)),
                       jnp.where(g1, i1, jnp.where(g2, idx, i2)))
        return top

    def select_tokens(top):
        vals = jnp.concatenate([top[0], top[2]], axis=0)
        ids = jnp.concatenate([top[1], top[3]], axis=0).astype(F32)
        big = float(S)
        m1 = jnp.max(vals)
        f1 = jnp.min(jnp.where(vals == m1, ids, big))
        vals2 = jnp.where(ids == f1, -jnp.inf, vals)
        m2 = jnp.max(vals2)
        f2 = jnp.min(jnp.where(jnp.logical_and(vals2 == m2, ids != f1), ids, big))
        i1 = jnp.minimum(f1.astype(jnp.int32), S - 1)
        i2 = jnp.minimum(f2.astype(jnp.int32), S - 1)
        idx_ref[0] = i1
        idx_ref[1] = i2
        sub = lax.broadcasted_iota(jnp.int32, (16, D), 0)

        def pick(ix):
            base = pl.multiple_of((ix // 16) * 16, 16)
            blk = xn_ref[pl.ds(base, 16), :].astype(F32)
            return jnp.sum(jnp.where(sub == ix - base, blk, 0.0), axis=0, keepdims=True)

        xs_ref[...] = jnp.where(sub == 0, pick(i1), jnp.where(sub == 1, pick(i2), 0.0)).astype(BF16)
        rs_ref[...] = jax.nn.sigmoid(jnp.where(sub == 0, m1, m2))

    def prep_k(slot):
        zz = jnp.zeros((PADW - DH, W), BF16)
        kp_ref[slot, 0] = jnp.concatenate([kt_buf[slot, 0], zz], axis=0).T
        kp_ref[slot, 1] = jnp.concatenate([zz, kt_buf[slot, 1]], axis=0).T

    def qproj_tile(u, n, slot):
        w = wq_buf[slot, :, n * LANE:(n + 1) * LANE]
        return (_nn_q(xn_ref[rows(u), :], w) * c).astype(BF16)

    def qproj_split(u, slot):
        parts = [(_nn_q(xn_ref[rows(u, t, 4), :], wq_buf[slot]) * c).astype(BF16) for t in range(4)]
        q = jnp.concatenate(parts, axis=0)
        return [q[:, n * LANE:(n + 1) * LANE] for n in range(3)]

    def qk(q, h, slot):
        st = _nt(kp_ref[slot, h], jnp.concatenate(q[h:h + 2], axis=1))
        s_refs[h][0] = st
        return jnp.max(st, axis=0, keepdims=True)

    def softmax(m, h):
        e = jnp.exp2(s_refs[h][z] - m)
        return e.astype(BF16), jnp.sum(e, axis=0, keepdims=True)

    def pv(p, l, h, slot, dep=None):
        one = 1.0 if dep is None else tie(dep[0:1, 0:1], 1.0)
        return (_nn_pv(vt_buf[slot, h], p) * (one / l)).astype(BF16)

    def finish(u, val, n0, n1, part, nparts):
        r = rows(u, part, nparts)
        cs = slice(n0 * LANE, n1 * LANE)
        g = _silu(xg_ref[r, cs].astype(F32))
        out_buf[r, cs] = (x_buf[r, cs].astype(F32) + val * g).astype(out_buf.dtype)

    def finish_rows(u, chain):
        GR = 16
        for t in range(TQ // GR):
            r = pl.ds(u * TQ + t * GR, GR)
            gin = xg_ref[r, :].astype(F32)
            if GT > 0 and len(chain) >= GT:
                h = gin * tie(chain[-GT], 0.5)
            else:
                h = gin * 0.5
            g = h + h * jnp.tanh(h)
            o = x_buf[r, :].astype(F32) + acc_ref[r, :] * g
            chain.append(o[:, D - 1:D])
            out_buf[r, :] = o.astype(out_buf.dtype)

    def wo_cols(u, o, slot, n0, n1, part=0, nparts=1, final=False):
        n = TQ // nparts
        r = rows(u, part, nparts)
        cs = slice(n0 * LANE, n1 * LANE)
        val = acc_ref[r, cs] + _nn_wo(o[part * n:(part + 1) * n], wo_buf[slot, :, cs])
        if final:
            finish(u, val, n0, n1, part, nparts)
        else:
            acc_ref[r, cs] = val

    def unit(q, prev, bslot, a, cc, final=False, mid=None, dep=None):
        m0 = qk(q, 0, bslot)
        m1 = qk(q, 1, bslot)
        if mid is not None:
            mid()
        p0 = softmax(m0, 0)
        p1 = softmax(m1, 1)
        if cc is not None:
            o = prev.T
        if a is not None and cc is not None:
            qn = []
            for n in range(3):
                qn.append(qproj_tile(a[0], n, a[1]))
                wo_cols(cc[0], o, cc[1], n, n + 1, final=final)
            wo_cols(cc[0], o, cc[1], 3, 5, 0, 2, final=final)
            wo_cols(cc[0], o, cc[1], 3, 5, 1, 2, final=final)
        elif a is not None:
            qn = qproj_split(a[0], a[1])
        else:
            qn = None
            for t in range(4):
                wo_cols(cc[0], o, cc[1], 0, 5, t, 4, final=final)
        o0 = pv(*p0, 0, bslot, dep)
        o1 = pv(*p1, 1, bslot)
        return qn, jnp.concatenate([o0, o1], axis=0)

    def load_carry():
        qv = q_st[...]
        return [qv[:, n * LANE:(n + 1) * LANE] for n in range(3)], ot_st[...]

    def store_carry(q, prev):
        q_st[...] = jnp.concatenate(q, axis=1)
        ot_st[...] = prev

    def sync(starts=(), waits=()):
        def body(i, carry):
            for cp, prio in starts:
                cp.start(priority=prio)
            for cp in waits:
                cp.wait()
            return carry
        lax.fori_loop(0, z + 1, body, 0)

    def prologue():
        cp_wr = pltpu.make_async_copy(wr_hbm, wr_ref, sem_f.at[3])
        cp_wr.start()
        cp_x(0).start()
        cp_wq(0).start(priority=1)
        cp_k(0).start(priority=1)
        cp_x(1).start(priority=1)
        cp_v(0).start(priority=1)
        with scope("w_x0"):
            cp_x(0).wait()
            cp_wr.wait()
        with scope("ln0"):
            top = layernorm(0, None)
        with scope("w_wq0"):
            sync([(cp_x(2), 1), (cp_x(3), 1), (cp_wo(0), 1)], [cp_wq(0)])
        with scope("a0"):
            parts = [(_nn_q(xn_ref[rows(0, t, 4), :], wq_buf[0]) * c).astype(BF16) for t in range(2)]
        with scope("w_k0"):
            sync([], [cp_k(0)])
        with scope("a0b"):
            parts += [(_nn_q(xn_ref[rows(0, t, 4), :], wq_buf[0]) * c).astype(BF16) for t in range(2, 4)]
            prep_k(0)
            qv = jnp.concatenate(parts, axis=0)
            q = [qv[:, n * LANE:(n + 1) * LANE] for n in range(3)]
        with scope("w1"):
            sync([(cp_x(t), 1) for t in range(4, U)] + [(cp_k(1), 1)], [cp_x(1), cp_v(0)])
        prev = None
        plan = {0: [1], 1: [2, 3], 2: [4, 5], 3: [6, 7]}
        for u in range(R):
            if u == 1:
                with scope("w3"):
                    sync([(cp, 1) for cp in cp_pair(1)] + [(cp_k(2), 1)], [cp_x(2), cp_x(3), cp_wo(0)])
            if u == 2:
                with scope("w4"):
                    sync([(cp, 1) for cp in cp_pair(2)] + [(cp_k(3), 1)] + [(cp, 1) for cp in cp_ffn()],
                         [cp_x(t) for t in range(4, U)] + [cp_k(1)])
            with scope("unit" if u < 2 else "unit23") if u != 3 else contextlib.nullcontext():
                if u != 3:
                    chain = []
                for t in plan[u]:
                    top = layernorm(t, top, chain if G > 0 else None)
                q, prev = unit(q, prev, 0, (u + 1, 0), (u - 1, 0) if u > 0 else None,
                               mid=(lambda: prep_k(1)) if u == R - 1 else None)
        assert R == 4 and U == 8
        store_carry(q, prev)
        select_tokens(top)

    def ffn_block():
        for cp in cp_ffn():
            cp.wait()
        xs = xs_ref[...]
        gg = _nn(xs, wg_ref[...])
        uu = _nn(xs, wu_ref[...])
        hmid = (_silu(gg) * uu).astype(BF16)
        y = _nn(hmid, wd_ref[...]) * rs_ref[...]
        sub = lax.broadcasted_iota(jnp.int32, (16, D), 0)
        for k in range(2):
            ix = idx_ref[k]
            base = pl.multiple_of((ix // 16) * 16, 16)
            blk = xg_ref[pl.ds(base, 16), :].astype(F32)
            xg_ref[pl.ds(base, 16), :] = jnp.where(sub == ix - base, blk + y[k:k + 1, :], blk).astype(BF16)

    def main(j):
        s0 = slot_of(j)
        s1 = slot_of(j + 1)
        s2 = slot_of(j + 2)
        for cp in cp_pair(j + 1):
            cp.wait()

        @pl.when(j + 2 < NP)
        def _():
            cp_k(j + 2).wait()

        q, prev = load_carry()
        for v in range(U):
            u = (R + v) % U
            bs = s1 if v >= U - R else s0
            as_ = s1 if v + 1 >= U - R else s0
            cs_ = s1 if v - 1 >= U - R else s0
            mid = (lambda: prep_k(s2)) if v == U - 1 else None
            q, prev = unit(q, prev, bs, ((u + 1) % U, as_), ((u - 1) % U, cs_), mid=mid)
        store_carry(q, prev)

        @pl.when(j + 3 < NP)
        def _():
            for cp in cp_pair(j + 3):
                cp.start()

        @pl.when(j + 4 < NP)
        def _():
            cp_k(j + 4).start()

    def tail():
        p = slot_of(NP - 1)
        q, prev = load_carry()
        early = list(range(R - 1))
        def fence_out():
            return out_buf[pl.ds(pl.multiple_of(z * 16, 16), 16), 0:LANE].astype(F32)

        chain = []
        dep = None
        for u in range(R, U):
            a = (u + 1, p) if u + 1 < U else None
            if early and (u - R) >= ESTART:
                e = early.pop(0)
                finish_rows(e, chain)
                cp_out(e).start()
                if FENCE & 1:
                    dep = fence_out()
            q, prev = unit(q, prev, p, a, (u - 1, p), final=True, dep=dep)
            cp_out(u - 1).start()
            dep = fence_out() if FENCE & 2 else None
        assert not early
        o = prev.T
        for t in range(4):
            wo_cols(U - 1, o, p, 0, 5, t, 4, final=True)
            cp_out(U - 1, t, 4).start()
        for t in range(U - 1):
            cp_out(t).wait()
        for t in range(4):
            cp_out(U - 1, t, 4).wait()

    if "P" in only:
        @pl.when(step == 0)
        def _():
            with scope("P"):
                prologue()

    if "F" in only:
        @pl.when(step == 2)
        def _():
            with scope("ffn"):
                ffn_block()

    if "M" in only:
        @pl.when(jnp.logical_and(step > 0, step < NP))
        def _():
            with scope("M"):
                main(step - 1)

    if "T" in only:
        @pl.when(step == NP)
        def _():
            with scope("T"):
                tail()


def _build(TQ=256, VMEM_MB=100, scopes=False, only="PFMT", R=4, G=4, RF32=True, GT=4, ESTART=0, FENCE=3):
    def fn(A_x, A_k_cache, A_v_cache, A_wq, A_wo, B_x, B_w_r, B_w_gate, B_w_up, B_w_down):
        B, S, D = A_x.shape
        _, H, SK, DH = A_k_cache.shape
        W = min(4096, max(256, SK // 4))
        assert B == 1 and H % 2 == 0
        NP = H // 2
        assert NP >= 4
        U = S // TQ
        FF = B_w_gate.shape[1]
        x = A_x.reshape(S, D)
        kern = functools.partial(_kernel, TQ=TQ, NP=NP, DH=DH, W=W, eps=1e-5, scopes=scopes, only=only, R=R, G=G, RF32=RF32, GT=GT, ESTART=ESTART, FENCE=FENCE)
        hbm = pl.BlockSpec(memory_space=pl.ANY)
        out = pl.pallas_call(
            kern,
            grid=(NP + 1,),
            in_specs=[hbm, hbm, hbm, hbm, hbm,
                      hbm,
                      hbm, hbm, hbm],
            out_specs=hbm,
            out_shape=jax.ShapeDtypeStruct((S, D), A_x.dtype),
            scratch_shapes=[
                pltpu.VMEM((S, D), BF16),
                pltpu.VMEM((S, D), BF16),
                pltpu.VMEM((S, D), BF16),
                pltpu.VMEM((S, D), F32),
                pltpu.VMEM((S, D), A_x.dtype),
                pltpu.VMEM((NSLOT, D, 2 * DH), BF16),
                pltpu.VMEM((NSLOT, 2 * DH, D), BF16),
                pltpu.VMEM((NSLOT, 2, DH, W), BF16),
                pltpu.VMEM((NSLOT, 2, DH, W), BF16),
                pltpu.VMEM((NSLOT, 2, W, 2 * LANE), BF16),
                pltpu.VMEM((TQ, 2 * DH), BF16),
                pltpu.VMEM((2 * DH, TQ), BF16),
                pltpu.VMEM((1, W, TQ), F32),
                pltpu.VMEM((1, W, TQ), F32),
                pltpu.VMEM((16, D), BF16),
                pltpu.VMEM((16, D), F32),
                pltpu.SMEM((2,), jnp.int32),
                pltpu.VMEM((D,), BF16),
                pltpu.VMEM((D, FF), BF16),
                pltpu.VMEM((D, FF), BF16),
                pltpu.VMEM((FF, D), BF16),
                pltpu.SemaphoreType.DMA((U,)),
                pltpu.SemaphoreType.DMA((NSLOT,)),
                pltpu.SemaphoreType.DMA((NSLOT,)),
                pltpu.SemaphoreType.DMA((NSLOT,)),
                pltpu.SemaphoreType.DMA((NSLOT,)),
                pltpu.SemaphoreType.DMA((4,)),
                pltpu.SemaphoreType.DMA((U + 3,)),
            ],
            compiler_params=pltpu.CompilerParams(
                dimension_semantics=("arbitrary",),
                vmem_limit_bytes=VMEM_MB * 1024 * 1024),
            name="fused_attn_moe",
        )(x, jnp.swapaxes(A_k_cache, 2, 3), jnp.swapaxes(A_v_cache, 2, 3), A_wq, A_wo, B_w_r,
          B_w_gate, B_w_up, B_w_down)
        return out.reshape(B, S, D)
    return fn


@jax.jit
def pallas_recurrent_scan__sliding_block_cached__moe_arch_mod__prompt_kernel(
        A_x, A_k_cache, A_v_cache, A_wq, A_wo, B_x, B_w_r, B_w_gate, B_w_up, B_w_down):
    return _build()(A_x, A_k_cache, A_v_cache, A_wq, A_wo, B_x, B_w_r, B_w_gate, B_w_up, B_w_down)
```

```python
import functools
import math

import jax
import jax.numpy as jnp
from jax import lax
import jax.experimental.pallas as pl
import jax.experimental.pallas.tpu as pltpu

F32 = jnp.float32
BF16 = jnp.bfloat16
LANE = 128
SUB = 8
NSLOT = 4
TQ = 256
R = 4
G_LN = 6
G_FIN = 3


def _nt(a, b):
    return lax.dot_general(a, b, (((1,), (1,)), ((), ())), preferred_element_type=F32)


def _nn(a, b):
    return jnp.dot(a, b, preferred_element_type=F32)


def _silu(x):
    h = 0.5 * x
    return h + h * jnp.tanh(h)


def _kernel(x_hbm, kt_hbm, vt_hbm, wq_hbm, wo_hbm, wr_hbm, wg_hbm, wu_hbm, wd_hbm,
            out_hbm,
            x_buf, xn_ref, xg_ref, acc_ref, out_buf, wq_buf, wo_buf, kt_buf, vt_buf, kp_ref,
            q_st, ot_st, s0_ref, s1_ref, xs_ref, rs_ref, idx_ref, wr_ref, wg_ref, wu_ref, wd_ref,
            sem_x, sem_wq, sem_wo, sem_k, sem_v, sem_f, sem_o,
            *, NP, DH, W, eps):
    S, D = x_buf.shape
    U = S // TQ
    PW = 2 * DH
    PADW = 2 * LANE
    SK = kt_hbm.shape[-1]
    c = (DH ** -0.5) * math.log2(math.e)
    step = pl.program_id(0)
    z = lax.shift_right_logical(step, (NP + 1).bit_length())
    s_refs = (s0_ref, s1_ref)

    def slot_of(p):
        return p % NSLOT if isinstance(p, int) else p & (NSLOT - 1)

    def rows(u, part=0, nparts=1):
        n = TQ // nparts
        return pl.ds(u * TQ + part * n, n)

    def cp_x(t):
        return pltpu.make_async_copy(x_hbm.at[pl.ds(t * TQ, TQ)], x_buf.at[pl.ds(t * TQ, TQ)], sem_x.at[t])

    def col(p):
        return p * PW if isinstance(p, int) else pl.multiple_of(p * PW, LANE)

    def cp_wq(p):
        s = slot_of(p)
        return pltpu.make_async_copy(wq_hbm.at[:, pl.ds(col(p), PW)], wq_buf.at[s], sem_wq.at[s])

    def cp_wo(p):
        s = slot_of(p)
        return pltpu.make_async_copy(wo_hbm.at[pl.ds(col(p), PW)], wo_buf.at[s], sem_wo.at[s])

    def cp_k(p):
        s = slot_of(p)
        return pltpu.make_async_copy(kt_hbm.at[0, pl.ds(2 * p, 2), :, pl.ds(SK - W, W)], kt_buf.at[s], sem_k.at[s])

    def cp_v(p):
        s = slot_of(p)
        return pltpu.make_async_copy(vt_hbm.at[0, pl.ds(2 * p, 2), :, pl.ds(SK - W, W)], vt_buf.at[s], sem_v.at[s])

    def cp_pair(p):
        return (cp_wq(p), cp_v(p), cp_wo(p))

    def cp_ffn():
        return (pltpu.make_async_copy(wg_hbm, wg_ref, sem_f.at[0]),
                pltpu.make_async_copy(wu_hbm, wu_ref, sem_f.at[1]),
                pltpu.make_async_copy(wd_hbm, wd_ref, sem_f.at[2]))

    def cp_out(t, part=0, nparts=1):
        r = rows(t, part, nparts)
        return pltpu.make_async_copy(out_buf.at[r], out_hbm.at[r], sem_o.at[t + part])

    def tie(v, const):
        cb = lax.bitcast_convert_type(jnp.float32(const), jnp.int32)
        vb = lax.bitcast_convert_type(v, jnp.int32)
        return lax.bitcast_convert_type(jnp.minimum((vb & 0x7FFFFFFF) | cb, cb), F32)

    def layernorm(u, top, chain=None):
        GR = 16
        wr = wr_ref[...].astype(F32).reshape(1, D)
        sub = lax.broadcasted_iota(jnp.int32, (SUB, LANE), 0)
        acc_ref[rows(u), :] = jnp.zeros((TQ, D), F32)
        for t in range(TQ // GR):
            r = pl.ds(u * TQ + t * GR, GR)
            x = x_buf[r, :].astype(F32)
            ssum = jnp.sum(x, axis=-1, keepdims=True)
            if chain is not None and len(chain) >= G_LN:
                m = ssum * tie(chain[-G_LN], 1.0 / D)
            else:
                m = ssum * (1.0 / D)
            xc = x - m
            v = jnp.sum(xc * xc, axis=-1, keepdims=True) * (1.0 / D)
            xf = xc * lax.rsqrt(v + eps)
            xn = xf.astype(BF16)
            xn_ref[r, :] = xn
            xg_ref[r, :] = xn
            sc = jnp.sum(xf * wr, axis=-1, keepdims=True)
            sc = sc.astype(BF16).astype(F32)
            if chain is not None:
                chain.append(sc)
            scb = jnp.broadcast_to(sc, (GR, LANE))
            for h in range(GR // SUB):
                val = scb[h * SUB:(h + 1) * SUB]
                idx = sub + (u * TQ + t * GR + h * SUB)
                if top is None:
                    top = (val, idx, jnp.full((SUB, LANE), -jnp.inf, F32), idx)
                    continue
                m1, i1, m2, i2 = top
                g1 = val > m1
                g2 = val > m2
                top = (jnp.where(g1, val, m1), jnp.where(g1, idx, i1),
                       jnp.where(g1, m1, jnp.where(g2, val, m2)),
                       jnp.where(g1, i1, jnp.where(g2, idx, i2)))
        return top

    def select_tokens(top):
        vals = jnp.concatenate([top[0], top[2]], axis=0)
        ids = jnp.concatenate([top[1], top[3]], axis=0).astype(F32)
        big = float(S)
        m1 = jnp.max(vals)
        f1 = jnp.min(jnp.where(vals == m1, ids, big))
        vals2 = jnp.where(ids == f1, -jnp.inf, vals)
        m2 = jnp.max(vals2)
        f2 = jnp.min(jnp.where(jnp.logical_and(vals2 == m2, ids != f1), ids, big))
        i1 = jnp.minimum(f1.astype(jnp.int32), S - 1)
        i2 = jnp.minimum(f2.astype(jnp.int32), S - 1)
        idx_ref[0] = i1
        idx_ref[1] = i2
        sub = lax.broadcasted_iota(jnp.int32, (16, D), 0)

        def pick(ix):
            base = pl.multiple_of((ix // 16) * 16, 16)
            blk = xn_ref[pl.ds(base, 16), :].astype(F32)
            return jnp.sum(jnp.where(sub == ix - base, blk, 0.0), axis=0, keepdims=True)

        xs_ref[...] = jnp.where(sub == 0, pick(i1), jnp.where(sub == 1, pick(i2), 0.0)).astype(BF16)
        rs_ref[...] = jax.nn.sigmoid(jnp.where(sub == 0, m1, m2))

    def prep_k(slot):
        zz = jnp.zeros((PADW - DH, W), BF16)
        kp_ref[slot, 0] = jnp.concatenate([kt_buf[slot, 0], zz], axis=0).T
        kp_ref[slot, 1] = jnp.concatenate([zz, kt_buf[slot, 1]], axis=0).T

    def qproj_tile(u, n, slot):
        w = wq_buf[slot, :, n * LANE:(n + 1) * LANE]
        return (_nn(xn_ref[rows(u), :], w) * c).astype(BF16)

    def qproj_quarter(u, t, slot):
        return (_nn(xn_ref[rows(u, t, 4), :], wq_buf[slot]) * c).astype(BF16)

    def split_tiles(qv):
        return [qv[:, n * LANE:(n + 1) * LANE] for n in range(3)]

    def qk(q, h, slot):
        st = _nt(kp_ref[slot, h], jnp.concatenate(q[h:h + 2], axis=1))
        s_refs[h][0] = st
        return jnp.max(st, axis=0, keepdims=True)

    def softmax(m, h):
        e = jnp.exp2(s_refs[h][z] - m)
        return e.astype(BF16), jnp.sum(e, axis=0, keepdims=True)

    def pv(p, l, h, slot, dep=None):
        one = 1.0 if dep is None else tie(dep[0:1, 0:1], 1.0)
        return (_nn(vt_buf[slot, h], p) * (one / l)).astype(BF16)

    def finish(u, val, n0, n1, part, nparts):
        r = rows(u, part, nparts)
        cs = slice(n0 * LANE, n1 * LANE)
        g = _silu(xg_ref[r, cs].astype(F32))
        out_buf[r, cs] = (x_buf[r, cs].astype(F32) + val * g).astype(out_buf.dtype)

    def finish_rows(u, chain):
        GR = 16
        for t in range(TQ // GR):
            r = pl.ds(u * TQ + t * GR, GR)
            gin = xg_ref[r, :].astype(F32)
            if len(chain) >= G_FIN:
                h = gin * tie(chain[-G_FIN], 0.5)
            else:
                h = gin * 0.5
            g = h + h * jnp.tanh(h)
            o = x_buf[r, :].astype(F32) + acc_ref[r, :] * g
            chain.append(o[:, D - 1:D])
            out_buf[r, :] = o.astype(out_buf.dtype)

    def wo_cols(u, o, slot, n0, n1, part=0, nparts=1, final=False):
        n = TQ // nparts
        r = rows(u, part, nparts)
        cs = slice(n0 * LANE, n1 * LANE)
        val = acc_ref[r, cs] + _nn(o[part * n:(part + 1) * n], wo_buf[slot, :, cs])
        if final:
            finish(u, val, n0, n1, part, nparts)
        else:
            acc_ref[r, cs] = val

    def unit(q, prev, bslot, a, cc, final=False, mid=None, dep0=None, dep1=None):
        m0 = qk(q, 0, bslot)
        m1 = qk(q, 1, bslot)
        if mid is not None:
            mid()
        p0 = softmax(m0, 0)
        p1 = softmax(m1, 1)
        if cc is not None:
            o = prev.T
        if a is not None and cc is not None:
            qn = []
            for n in range(3):
                qn.append(qproj_tile(a[0], n, a[1]))
                wo_cols(cc[0], o, cc[1], n, n + 1, final=final)
            wo_cols(cc[0], o, cc[1], 3, 5, 0, 2, final=final)
            wo_cols(cc[0], o, cc[1], 3, 5, 1, 2, final=final)
        elif a is not None:
            qn = split_tiles(jnp.concatenate([qproj_quarter(a[0], t, a[1]) for t in range(4)], axis=0))
        else:
            qn = None
            for t in range(4):
                wo_cols(cc[0], o, cc[1], 0, 5, t, 4, final=final)
        o0 = pv(*p0, 0, bslot, dep0)
        o1 = pv(*p1, 1, bslot, dep1)
        return qn, jnp.concatenate([o0, o1], axis=0)

    def load_carry():
        return split_tiles(q_st[...]), ot_st[...]

    def store_carry(q, prev):
        q_st[...] = jnp.concatenate(q, axis=1)
        ot_st[...] = prev

    def sync(starts=(), waits=()):
        def body(i, carry):
            for cp in starts:
                cp.start(priority=1)
            for cp in waits:
                cp.wait()
            return carry
        lax.fori_loop(0, z + 1, body, 0)

    def prologue():
        cp_wr = pltpu.make_async_copy(wr_hbm, wr_ref, sem_f.at[3])
        cp_wr.start()
        cp_x(0).start()
        cp_wq(0).start(priority=1)
        cp_k(0).start(priority=1)
        cp_x(1).start(priority=1)
        cp_v(0).start(priority=1)
        cp_x(0).wait()
        cp_wr.wait()
        top = layernorm(0, None)
        sync([cp_x(2), cp_x(3), cp_wo(0)], [cp_wq(0)])
        parts = [qproj_quarter(0, t, 0) for t in range(2)]
        sync([], [cp_k(0)])
        parts += [qproj_quarter(0, t, 0) for t in range(2, 4)]
        prep_k(0)
        q = split_tiles(jnp.concatenate(parts, axis=0))
        sync([cp_x(t) for t in range(4, U)] + [cp_k(1)], [cp_x(1), cp_v(0)])
        prev = None
        plan = {0: [1], 1: [2, 3], 2: [4, 5], 3: [6, 7]}
        for u in range(R):
            if u == 1:
                sync(list(cp_pair(1)) + [cp_k(2)], [cp_x(2), cp_x(3), cp_wo(0)])
            if u == 2:
                sync(list(cp_pair(2)) + [cp_k(3)] + list(cp_ffn()), [cp_x(t) for t in range(4, U)] + [cp_k(1)])
            if u != 3:
                chain = []
            for t in plan[u]:
                top = layernorm(t, top, chain)
            q, prev = unit(q, prev, 0, (u + 1, 0), (u - 1, 0) if u > 0 else None,
                           mid=(lambda: prep_k(1)) if u == R - 1 else None,
                           dep1=chain[-1] if u >= 2 else None)
        store_carry(q, prev)
        select_tokens(top)

    def ffn_block():
        for cp in cp_ffn():
            cp.wait()
        xs = xs_ref[...]
        gg = _nn(xs, wg_ref[...])
        uu = _nn(xs, wu_ref[...])
        hmid = (_silu(gg) * uu).astype(BF16)
        y = _nn(hmid, wd_ref[...]) * rs_ref[...]
        sub = lax.broadcasted_iota(jnp.int32, (16, D), 0)
        for k in range(2):
            ix = idx_ref[k]
            base = pl.multiple_of((ix // 16) * 16, 16)
            blk = xg_ref[pl.ds(base, 16), :].astype(F32)
            xg_ref[pl.ds(base, 16), :] = jnp.where(sub == ix - base, blk + y[k:k + 1, :], blk).astype(BF16)

    def main(j):
        s0 = slot_of(j)
        s1 = slot_of(j + 1)
        s2 = slot_of(j + 2)
        for cp in cp_pair(j + 1):
            cp.wait()

        @pl.when(j + 2 < NP)
        def _():
            cp_k(j + 2).wait()

        q, prev = load_carry()
        for v in range(U):
            u = (R + v) % U
            bs = s1 if v >= U - R else s0
            as_ = s1 if v + 1 >= U - R else s0
            cs_ = s1 if v - 1 >= U - R else s0
            mid = (lambda: prep_k(s2)) if v == U - 1 else None
            q, prev = unit(q, prev, bs, ((u + 1) % U, as_), ((u - 1) % U, cs_), mid=mid)
        store_carry(q, prev)

        @pl.when(j + 3 < NP)
        def _():
            for cp in cp_pair(j + 3):
                cp.start()

        @pl.when(j + 4 < NP)
        def _():
            cp_k(j + 4).start()

    def tail():
        p = slot_of(NP - 1)
        q, prev = load_carry()
        early = list(range(R - 1))

        def fence_out():
            return out_buf[pl.ds(pl.multiple_of(z * 16, 16), 16), 0:LANE].astype(F32)

        chain = []
        dep = None
        for u in range(R, U):
            a = (u + 1, p) if u + 1 < U else None
            if early:
                e = early.pop(0)
                finish_rows(e, chain)
                cp_out(e).start()
                dep = fence_out()
            q, prev = unit(q, prev, p, a, (u - 1, p), final=True, dep0=dep)
            cp_out(u - 1).start()
            dep = fence_out() if u + 1 < U else None
        o = prev.T
        for t in range(4):
            wo_cols(U - 1, o, p, 0, 5, t, 4, final=True)
            cp_out(U - 1, t, 4).start()
        for t in range(U - 1):
            cp_out(t).wait()
        for t in range(4):
            cp_out(U - 1, t, 4).wait()

    pl.when(step == 0)(prologue)
    pl.when(step == 2)(ffn_block)
    pl.when(jnp.logical_and(step > 0, step < NP))(lambda: main(step - 1))
    pl.when(step == NP)(tail)


@jax.jit
def pallas_recurrent_scan__sliding_block_cached__moe_arch_mod__prompt_kernel(
        A_x, A_k_cache, A_v_cache, A_wq, A_wo, B_x, B_w_r, B_w_gate, B_w_up, B_w_down):
    B, S, D = A_x.shape
    _, H, SK, DH = A_k_cache.shape
    W = min(4096, max(256, SK // 4))
    NP = H // 2
    U = S // TQ
    FF = B_w_gate.shape[1]
    assert B == 1 and H % 2 == 0 and NP >= 4 and U == 8 and D == 5 * LANE and 2 * DH == 3 * LANE and W <= SK
    kern = functools.partial(_kernel, NP=NP, DH=DH, W=W, eps=1e-5)
    hbm = pl.BlockSpec(memory_space=pl.ANY)
    out = pl.pallas_call(
        kern,
        grid=(NP + 1,),
        in_specs=[hbm] * 9,
        out_specs=hbm,
        out_shape=jax.ShapeDtypeStruct((S, D), A_x.dtype),
        scratch_shapes=[
            pltpu.VMEM((S, D), BF16),
            pltpu.VMEM((S, D), BF16),
            pltpu.VMEM((S, D), BF16),
            pltpu.VMEM((S, D), F32),
            pltpu.VMEM((S, D), A_x.dtype),
            pltpu.VMEM((NSLOT, D, 2 * DH), BF16),
            pltpu.VMEM((NSLOT, 2 * DH, D), BF16),
            pltpu.VMEM((NSLOT, 2, DH, W), BF16),
            pltpu.VMEM((NSLOT, 2, DH, W), BF16),
            pltpu.VMEM((NSLOT, 2, W, 2 * LANE), BF16),
            pltpu.VMEM((TQ, 2 * DH), BF16),
            pltpu.VMEM((2 * DH, TQ), BF16),
            pltpu.VMEM((1, W, TQ), F32),
            pltpu.VMEM((1, W, TQ), F32),
            pltpu.VMEM((16, D), BF16),
            pltpu.VMEM((16, D), F32),
            pltpu.SMEM((2,), jnp.int32),
            pltpu.VMEM((D,), BF16),
            pltpu.VMEM((D, FF), BF16),
            pltpu.VMEM((D, FF), BF16),
            pltpu.VMEM((FF, D), BF16),
            pltpu.SemaphoreType.DMA((U,)),
            pltpu.SemaphoreType.DMA((NSLOT,)),
            pltpu.SemaphoreType.DMA((NSLOT,)),
            pltpu.SemaphoreType.DMA((NSLOT,)),
            pltpu.SemaphoreType.DMA((NSLOT,)),
            pltpu.SemaphoreType.DMA((4,)),
            pltpu.SemaphoreType.DMA((U + 3,)),
        ],
        compiler_params=pltpu.CompilerParams(
            dimension_semantics=("arbitrary",),
            vmem_limit_bytes=100 * 1024 * 1024,
            disable_bounds_checks=True,
            disable_semaphore_checks=True),
        name="fused_attn_moe",
    )(A_x.reshape(S, D), jnp.swapaxes(A_k_cache, 2, 3), jnp.swapaxes(A_v_cache, 2, 3), A_wq, A_wo, B_w_r,
      B_w_gate, B_w_up, B_w_down)
    return out.reshape(B, S, D)
```

```python
import functools
import math

import jax
import jax.numpy as jnp
from jax import lax
import jax.experimental.pallas as pl
import jax.experimental.pallas.tpu as pltpu

F32 = jnp.float32
BF16 = jnp.bfloat16
LANE = 128
SUB = 8
NSLOT = 4
TQ = 256
R = 4
G_LN = 6
G_FIN = 3


def _nt(a, b):
    return lax.dot_general(a, b, (((1,), (1,)), ((), ())), preferred_element_type=F32)


def _nn(a, b):
    return jnp.dot(a, b, preferred_element_type=F32)


def _silu(x):
    h = 0.5 * x
    return h + h * jnp.tanh(h)


def _kernel(x_hbm, kt_hbm, vt_hbm, wq_hbm, wo_hbm, wr_hbm, wg_hbm, wu_hbm, wd_hbm,
            out_hbm,
            x_buf, xn_ref, xg_ref, acc_ref, out_buf, wq_buf, wo_buf, kt_buf, vt_buf, kp_ref,
            q_st, ot_st, s0_ref, s1_ref, xs_ref, rs_ref, idx_ref, wr_ref, wg_ref, wu_ref, wd_ref,
            sem_x, sem_wq, sem_wo, sem_k, sem_v, sem_f, sem_o,
            *, NP, DH, W, eps):
    S, D = x_buf.shape
    U = S // TQ
    PW = 2 * DH
    PADW = 2 * LANE
    SK = kt_hbm.shape[-1]
    c = (DH ** -0.5) * math.log2(math.e)
    step = pl.program_id(0)
    z = lax.shift_right_logical(step, (NP + 1).bit_length())
    s_refs = (s0_ref, s1_ref)

    def slot_of(p):
        return p % NSLOT if isinstance(p, int) else p & (NSLOT - 1)

    def rows(u, part=0, nparts=1):
        n = TQ // nparts
        return pl.ds(u * TQ + part * n, n)

    def cp_x(t):
        return pltpu.make_async_copy(x_hbm.at[pl.ds(t * TQ, TQ)], x_buf.at[pl.ds(t * TQ, TQ)], sem_x.at[t])

    def col(p):
        return p * PW if isinstance(p, int) else pl.multiple_of(p * PW, LANE)

    def cp_wq(p):
        s = slot_of(p)
        return pltpu.make_async_copy(wq_hbm.at[:, pl.ds(col(p), PW)], wq_buf.at[s], sem_wq.at[s])

    def cp_wo(p):
        s = slot_of(p)
        return pltpu.make_async_copy(wo_hbm.at[pl.ds(col(p), PW)], wo_buf.at[s], sem_wo.at[s])

    def cp_k(p):
        s = slot_of(p)
        return pltpu.make_async_copy(kt_hbm.at[0, pl.ds(2 * p, 2), :, pl.ds(SK - W, W)], kt_buf.at[s], sem_k.at[s])

    def cp_v(p):
        s = slot_of(p)
        return pltpu.make_async_copy(vt_hbm.at[0, pl.ds(2 * p, 2), :, pl.ds(SK - W, W)], vt_buf.at[s], sem_v.at[s])

    def cp_pair(p):
        return (cp_wq(p), cp_v(p), cp_wo(p))

    def cp_ffn():
        return (pltpu.make_async_copy(wg_hbm, wg_ref, sem_f.at[0]),
                pltpu.make_async_copy(wu_hbm, wu_ref, sem_f.at[1]),
                pltpu.make_async_copy(wd_hbm, wd_ref, sem_f.at[2]))

    def cp_out(t, part=0, nparts=1):
        r = rows(t, part, nparts)
        return pltpu.make_async_copy(out_buf.at[r], out_hbm.at[r], sem_o.at[t + part])

    def tie(v, const):
        cb = lax.bitcast_convert_type(jnp.float32(const), jnp.int32)
        vb = lax.bitcast_convert_type(v, jnp.int32)
        return lax.bitcast_convert_type(jnp.minimum((vb & 0x7FFFFFFF) | cb, cb), F32)

    def layernorm(u, top, chain=None):
        GR = 16
        wr = wr_ref[...].astype(F32).reshape(1, D)
        sub = lax.broadcasted_iota(jnp.int32, (SUB, LANE), 0)
        acc_ref[rows(u), :] = jnp.zeros((TQ, D), F32)
        for t in range(TQ // GR):
            r = pl.ds(u * TQ + t * GR, GR)
            x = x_buf[r, :].astype(F32)
            ssum = jnp.sum(x, axis=-1, keepdims=True)
            if chain is not None and len(chain) >= G_LN:
                m = ssum * tie(chain[-G_LN], 1.0 / D)
            else:
                m = ssum * (1.0 / D)
            xc = x - m
            v = jnp.sum(xc * xc, axis=-1, keepdims=True) * (1.0 / D)
            xf = xc * lax.rsqrt(v + eps)
            xn = xf.astype(BF16)
            xn_ref[r, :] = xn
            xg_ref[r, :] = xn
            sc = jnp.sum(xf * wr, axis=-1, keepdims=True)
            sc = sc.astype(BF16).astype(F32)
            if chain is not None:
                chain.append(sc)
            scb = jnp.broadcast_to(sc, (GR, LANE))
            for h in range(GR // SUB):
                val = scb[h * SUB:(h + 1) * SUB]
                idx = sub + (u * TQ + t * GR + h * SUB)
                if top is None:
                    top = (val, idx, jnp.full((SUB, LANE), -jnp.inf, F32), idx)
                    continue
                m1, i1, m2, i2 = top
                g1 = val > m1
                g2 = val > m2
                top = (jnp.where(g1, val, m1), jnp.where(g1, idx, i1),
                       jnp.where(g1, m1, jnp.where(g2, val, m2)),
                       jnp.where(g1, i1, jnp.where(g2, idx, i2)))
        return top

    def select_tokens(top):
        vals = jnp.concatenate([top[0], top[2]], axis=0)
        ids = jnp.concatenate([top[1], top[3]], axis=0).astype(F32)
        big = float(S)
        m1 = jnp.max(vals)
        f1 = jnp.min(jnp.where(vals == m1, ids, big))
        vals2 = jnp.where(ids == f1, -jnp.inf, vals)
        m2 = jnp.max(vals2)
        f2 = jnp.min(jnp.where(jnp.logical_and(vals2 == m2, ids != f1), ids, big))
        i1 = jnp.minimum(f1.astype(jnp.int32), S - 1)
        i2 = jnp.minimum(f2.astype(jnp.int32), S - 1)
        idx_ref[0] = i1
        idx_ref[1] = i2
        sub = lax.broadcasted_iota(jnp.int32, (16, D), 0)

        def pick(ix):
            base = pl.multiple_of((ix // 16) * 16, 16)
            blk = xn_ref[pl.ds(base, 16), :].astype(F32)
            return jnp.sum(jnp.where(sub == ix - base, blk, 0.0), axis=0, keepdims=True)

        xs_ref[...] = jnp.where(sub == 0, pick(i1), jnp.where(sub == 1, pick(i2), 0.0)).astype(BF16)
        rs_ref[...] = jax.nn.sigmoid(jnp.where(sub == 0, m1, m2))

    def prep_k(slot):
        zz = jnp.zeros((PADW - DH, W), BF16)
        kp_ref[slot, 0] = jnp.concatenate([kt_buf[slot, 0], zz], axis=0).T
        kp_ref[slot, 1] = jnp.concatenate([zz, kt_buf[slot, 1]], axis=0).T

    def qproj_tile(u, n, slot):
        w = wq_buf[slot, :, n * LANE:(n + 1) * LANE]
        return (_nn(xn_ref[rows(u), :], w) * c).astype(BF16)

    def qproj_quarter(u, t, slot):
        return (_nn(xn_ref[rows(u, t, 4), :], wq_buf[slot]) * c).astype(BF16)

    def split_tiles(qv):
        return [qv[:, n * LANE:(n + 1) * LANE] for n in range(3)]

    def qk(q, h, slot):
        st = _nt(kp_ref[slot, h], jnp.concatenate(q[h:h + 2], axis=1))
        s_refs[h][0] = st
        return jnp.max(st, axis=0, keepdims=True)

    def softmax(m, h):
        e = jnp.exp2(s_refs[h][z] - m)
        return e.astype(BF16), jnp.sum(e, axis=0, keepdims=True)

    def pv(p, l, h, slot, dep=None):
        one = 1.0 if dep is None else tie(dep[0:1, 0:1], 1.0)
        return (_nn(vt_buf[slot, h], p) * (one / l)).astype(BF16)

    def finish(u, val, n0, n1, part, nparts):
        r = rows(u, part, nparts)
        cs = slice(n0 * LANE, n1 * LANE)
        g = _silu(xg_ref[r, cs].astype(F32))
        out_buf[r, cs] = (x_buf[r, cs].astype(F32) + val * g).astype(out_buf.dtype)

    def finish_rows(u, chain):
        GR = 16
        for t in range(TQ // GR):
            r = pl.ds(u * TQ + t * GR, GR)
            gin = xg_ref[r, :].astype(F32)
            if len(chain) >= G_FIN:
                h = gin * tie(chain[-G_FIN], 0.5)
            else:
                h = gin * 0.5
            g = h + h * jnp.tanh(h)
            o = x_buf[r, :].astype(F32) + acc_ref[r, :] * g
            chain.append(o[:, D - 1:D])
            out_buf[r, :] = o.astype(out_buf.dtype)

    def wo_cols(u, o, slot, n0, n1, part=0, nparts=1, final=False):
        n = TQ // nparts
        r = rows(u, part, nparts)
        cs = slice(n0 * LANE, n1 * LANE)
        val = acc_ref[r, cs] + _nn(o[part * n:(part + 1) * n], wo_buf[slot, :, cs])
        if final:
            finish(u, val, n0, n1, part, nparts)
        else:
            acc_ref[r, cs] = val

    def unit(q, prev, bslot, a, cc, final=False, mid=None, dep0=None, dep1=None):
        m0 = qk(q, 0, bslot)
        m1 = qk(q, 1, bslot)
        if mid is not None:
            mid()
        p0 = softmax(m0, 0)
        p1 = softmax(m1, 1)
        o = prev.T
        if a is not None:
            qn = []
            for n in range(3):
                qn.append(qproj_tile(a[0], n, a[1]))
                wo_cols(cc[0], o, cc[1], n, n + 1, final=final)
            wo_cols(cc[0], o, cc[1], 3, 5, 0, 2, final=final)
            wo_cols(cc[0], o, cc[1], 3, 5, 1, 2, final=final)
        else:
            qn = None
            for t in range(4):
                wo_cols(cc[0], o, cc[1], 0, 5, t, 4, final=final)
        o0 = pv(*p0, 0, bslot, dep0)
        o1 = pv(*p1, 1, bslot, dep1)
        return qn, jnp.concatenate([o0, o1], axis=0)

    def load_carry():
        return split_tiles(q_st[...]), ot_st[...]

    def store_carry(q, prev):
        q_st[...] = jnp.concatenate(q, axis=1)
        ot_st[...] = prev

    def sync(starts=(), waits=()):
        def body(i, carry):
            for cp in starts:
                cp.start(priority=1)
            for cp in waits:
                cp.wait()
            return carry
        lax.fori_loop(0, z + 1, body, 0)

    def prologue():
        cp_wr = pltpu.make_async_copy(wr_hbm, wr_ref, sem_f.at[3])
        cp_wr.start()
        cp_x(0).start()
        cp_wq(0).start(priority=1)
        cp_k(0).start(priority=1)
        cp_x(1).start(priority=1)
        cp_v(0).start(priority=1)
        cp_x(0).wait()
        cp_wr.wait()
        top = layernorm(0, None)
        sync([cp_x(2), cp_wo(0), cp_x(3)], [cp_wq(0)])
        parts = [qproj_quarter(0, t, 0) for t in range(2)]
        sync([], [cp_k(0)])
        parts += [qproj_quarter(0, t, 0) for t in range(2, 4)]
        prep_k(0)
        q = split_tiles(jnp.concatenate(parts, axis=0))
        sync([cp_x(t) for t in range(4, U)] + [cp_k(1)], [cp_x(1)])
        top = layernorm(1, top, [])
        m0 = qk(q, 0, 0)
        m1 = qk(q, 1, 0)
        p0 = softmax(m0, 0)
        p1 = softmax(m1, 1)
        q = split_tiles(jnp.concatenate([qproj_quarter(1, t, 0) for t in range(4)], axis=0))
        plan = {1: [2], 2: [3, 4, 5], 3: [6, 7]}
        sync(list(cp_pair(1)) + [cp_k(2)], [cp_v(0), cp_wo(0), cp_x(2)])
        prev = jnp.concatenate([pv(*p0, 0, 0), pv(*p1, 1, 0)], axis=0)
        for u in range(1, R):
            if u == 2:
                sync(list(cp_pair(2)) + [cp_k(3)] + list(cp_ffn()), [cp_x(t) for t in range(3, U)] + [cp_k(1)])
            if u != 3:
                chain = []
            for t in plan[u]:
                top = layernorm(t, top, chain)
            q, prev = unit(q, prev, 0, (u + 1, 0), (u - 1, 0),
                           mid=(lambda: prep_k(1)) if u == R - 1 else None,
                           dep1=chain[-1] if u >= 2 else None)
        store_carry(q, prev)
        select_tokens(top)

    def ffn_block():
        for cp in cp_ffn():
            cp.wait()
        xs = xs_ref[...]
        gg = _nn(xs, wg_ref[...])
        uu = _nn(xs, wu_ref[...])
        hmid = (_silu(gg) * uu).astype(BF16)
        y = _nn(hmid, wd_ref[...]) * rs_ref[...]
        sub = lax.broadcasted_iota(jnp.int32, (16, D), 0)
        for k in range(2):
            ix = idx_ref[k]
            base = pl.multiple_of((ix // 16) * 16, 16)
            blk = xg_ref[pl.ds(base, 16), :].astype(F32)
            xg_ref[pl.ds(base, 16), :] = jnp.where(sub == ix - base, blk + y[k:k + 1, :], blk).astype(BF16)

    def main(j):
        s0 = slot_of(j)
        s1 = slot_of(j + 1)
        s2 = slot_of(j + 2)
        for cp in cp_pair(j + 1):
            cp.wait()

        @pl.when(j + 2 < NP)
        def _():
            cp_k(j + 2).wait()

        q, prev = load_carry()
        for v in range(U):
            u = (R + v) % U
            bs = s1 if v >= U - R else s0
            as_ = s1 if v + 1 >= U - R else s0
            cs_ = s1 if v - 1 >= U - R else s0
            mid = (lambda: prep_k(s2)) if v == U - 1 else None
            q, prev = unit(q, prev, bs, ((u + 1) % U, as_), ((u - 1) % U, cs_), mid=mid)
        store_carry(q, prev)

        @pl.when(j + 3 < NP)
        def _():
            for cp in cp_pair(j + 3):
                cp.start()

        @pl.when(j + 4 < NP)
        def _():
            cp_k(j + 4).start()

    def tail():
        p = slot_of(NP - 1)
        q, prev = load_carry()
        early = list(range(R - 1))

        def fence_out():
            return out_buf[pl.ds(pl.multiple_of(z * 16, 16), 16), 0:LANE].astype(F32)

        chain = []
        dep = None
        for u in range(R, U):
            a = (u + 1, p) if u + 1 < U else None
            if early:
                e = early.pop(0)
                finish_rows(e, chain)
                cp_out(e).start()
                dep = fence_out()
            q, prev = unit(q, prev, p, a, (u - 1, p), final=True, dep0=dep)
            cp_out(u - 1).start()
            dep = fence_out() if u + 1 < U else None
        o = prev.T
        for t in range(4):
            wo_cols(U - 1, o, p, 0, 5, t, 4, final=True)
            cp_out(U - 1, t, 4).start()
        for t in range(U - 1):
            cp_out(t).wait()
        for t in range(4):
            cp_out(U - 1, t, 4).wait()

    pl.when(step == 0)(prologue)
    pl.when(step == 2)(ffn_block)
    pl.when(jnp.logical_and(step > 0, step < NP))(lambda: main(step - 1))
    pl.when(step == NP)(tail)


@jax.jit
def pallas_recurrent_scan__sliding_block_cached__moe_arch_mod__prompt_kernel(
        A_x, A_k_cache, A_v_cache, A_wq, A_wo, B_x, B_w_r, B_w_gate, B_w_up, B_w_down):
    B, S, D = A_x.shape
    _, H, SK, DH = A_k_cache.shape
    W = min(4096, max(256, SK // 4))
    NP = H // 2
    U = S // TQ
    FF = B_w_gate.shape[1]
    assert B == 1 and H % 2 == 0 and NP >= 4 and U == 8 and D == 5 * LANE and 2 * DH == 3 * LANE and W <= SK
    kern = functools.partial(_kernel, NP=NP, DH=DH, W=W, eps=1e-5)
    hbm = pl.BlockSpec(memory_space=pl.ANY)
    out = pl.pallas_call(
        kern,
        grid=(NP + 1,),
        in_specs=[hbm] * 9,
        out_specs=hbm,
        out_shape=jax.ShapeDtypeStruct((S, D), A_x.dtype),
        scratch_shapes=[
            pltpu.VMEM((S, D), BF16),
            pltpu.VMEM((S, D), BF16),
            pltpu.VMEM((S, D), BF16),
            pltpu.VMEM((S, D), F32),
            pltpu.VMEM((S, D), A_x.dtype),
            pltpu.VMEM((NSLOT, D, 2 * DH), BF16),
            pltpu.VMEM((NSLOT, 2 * DH, D), BF16),
            pltpu.VMEM((NSLOT, 2, DH, W), BF16),
            pltpu.VMEM((NSLOT, 2, DH, W), BF16),
            pltpu.VMEM((NSLOT, 2, W, 2 * LANE), BF16),
            pltpu.VMEM((TQ, 2 * DH), BF16),
            pltpu.VMEM((2 * DH, TQ), BF16),
            pltpu.VMEM((1, W, TQ), F32),
            pltpu.VMEM((1, W, TQ), F32),
            pltpu.VMEM((16, D), BF16),
            pltpu.VMEM((16, D), F32),
            pltpu.SMEM((2,), jnp.int32),
            pltpu.VMEM((D,), BF16),
            pltpu.VMEM((D, FF), BF16),
            pltpu.VMEM((D, FF), BF16),
            pltpu.VMEM((FF, D), BF16),
            pltpu.SemaphoreType.DMA((U,)),
            pltpu.SemaphoreType.DMA((NSLOT,)),
            pltpu.SemaphoreType.DMA((NSLOT,)),
            pltpu.SemaphoreType.DMA((NSLOT,)),
            pltpu.SemaphoreType.DMA((NSLOT,)),
            pltpu.SemaphoreType.DMA((4,)),
            pltpu.SemaphoreType.DMA((U + 3,)),
        ],
        compiler_params=pltpu.CompilerParams(
            dimension_semantics=("arbitrary",),
            vmem_limit_bytes=100 * 1024 * 1024,
            disable_bounds_checks=True,
            disable_semaphore_checks=True),
        name="fused_attn_moe",
    )(A_x.reshape(S, D), jnp.swapaxes(A_k_cache, 2, 3), jnp.swapaxes(A_v_cache, 2, 3), A_wq, A_wo, B_w_r,
      B_w_gate, B_w_up, B_w_down)
    return out.reshape(B, S, D)
```

```python
import functools
import math

import jax
import jax.numpy as jnp
from jax import lax
import jax.experimental.pallas as pl
import jax.experimental.pallas.tpu as pltpu

F32 = jnp.float32
BF16 = jnp.bfloat16
LANE = 128
SUB = 8
NSLOT = 4
TQ = 256
R = 4
G_LN = 6
G_FIN = 3


def _nt(a, b):
    return lax.dot_general(a, b, (((1,), (1,)), ((), ())), preferred_element_type=F32)


def _nn(a, b):
    return jnp.dot(a, b, preferred_element_type=F32)


def _silu(x):
    h = 0.5 * x
    return h + h * jnp.tanh(h)


def _kernel(x_hbm, kt_hbm, vt_hbm, wq_hbm, wo_hbm, wr_hbm, wg_hbm, wu_hbm, wd_hbm,
            out_hbm,
            x_buf, xn_ref, xg_ref, acc_ref, out_buf, wq_buf, wo_buf, kt_buf, vt_buf, kp_ref,
            q_st, ot_st, s0_ref, s1_ref, xs_ref, rs_ref, idx_ref, wr_ref, wg_ref, wu_ref, wd_ref,
            sem_x, sem_wq, sem_wo, sem_k, sem_v, sem_f, sem_o,
            *, NP, DH, W, eps):
    S, D = x_buf.shape
    U = S // TQ
    PW = 2 * DH
    PADW = 2 * LANE
    SK = kt_hbm.shape[-1]
    c = (DH ** -0.5) * math.log2(math.e)
    step = pl.program_id(0)
    z = lax.shift_right_logical(step, 1)
    s_refs = (s0_ref, s1_ref)

    def slot_of(p):
        return p % NSLOT if isinstance(p, int) else p & (NSLOT - 1)

    def rows(u, part=0, nparts=1):
        n = TQ // nparts
        return pl.ds(u * TQ + part * n, n)

    def cp_x(t):
        return pltpu.make_async_copy(x_hbm.at[pl.ds(t * TQ, TQ)], x_buf.at[pl.ds(t * TQ, TQ)], sem_x.at[t])

    def col(p):
        return p * PW if isinstance(p, int) else pl.multiple_of(p * PW, LANE)

    def cp_wq(p):
        s = slot_of(p)
        return pltpu.make_async_copy(wq_hbm.at[:, pl.ds(col(p), PW)], wq_buf.at[s], sem_wq.at[s])

    def cp_wo(p):
        s = slot_of(p)
        return pltpu.make_async_copy(wo_hbm.at[pl.ds(col(p), PW)], wo_buf.at[s], sem_wo.at[s])

    def cp_k(p):
        s = slot_of(p)
        return pltpu.make_async_copy(kt_hbm.at[0, pl.ds(2 * p, 2), :, pl.ds(SK - W, W)], kt_buf.at[s], sem_k.at[s])

    def cp_v(p):
        s = slot_of(p)
        return pltpu.make_async_copy(vt_hbm.at[0, pl.ds(2 * p, 2), :, pl.ds(SK - W, W)], vt_buf.at[s], sem_v.at[s])

    def cp_pair(p):
        return (cp_wq(p), cp_v(p), cp_wo(p))

    def cp_ffn():
        return (pltpu.make_async_copy(wg_hbm, wg_ref, sem_f.at[0]),
                pltpu.make_async_copy(wu_hbm, wu_ref, sem_f.at[1]),
                pltpu.make_async_copy(wd_hbm, wd_ref, sem_f.at[2]))

    def cp_out(t, part=0, nparts=1):
        r = rows(t, part, nparts)
        return pltpu.make_async_copy(out_buf.at[r], out_hbm.at[r], sem_o.at[t + part])

    def tie(v, const):
        cb = lax.bitcast_convert_type(jnp.float32(const), jnp.int32)
        vb = lax.bitcast_convert_type(v, jnp.int32)
        return lax.bitcast_convert_type(jnp.minimum((vb & 0x7FFFFFFF) | cb, cb), F32)

    def layernorm(u, top, chain=None):
        GR = 16
        wr = wr_ref[...].astype(F32).reshape(1, D)
        sub = lax.broadcasted_iota(jnp.int32, (SUB, LANE), 0)
        acc_ref[rows(u), :] = jnp.zeros((TQ, D), F32)
        for t in range(TQ // GR):
            r = pl.ds(u * TQ + t * GR, GR)
            x = x_buf[r, :].astype(F32)
            ssum = jnp.sum(x, axis=-1, keepdims=True)
            if chain is not None and len(chain) >= G_LN:
                m = ssum * tie(chain[-G_LN], 1.0 / D)
            else:
                m = ssum * (1.0 / D)
            xc = x - m
            v = jnp.sum(xc * xc, axis=-1, keepdims=True) * (1.0 / D)
            xf = xc * lax.rsqrt(v + eps)
            xn = xf.astype(BF16)
            xn_ref[r, :] = xn
            xg_ref[r, :] = xn
            sc = jnp.sum(xf * wr, axis=-1, keepdims=True)
            sc = sc.astype(BF16).astype(F32)
            if chain is not None:
                chain.append(sc)
            scb = jnp.broadcast_to(sc, (GR, LANE))
            for h in range(GR // SUB):
                val = scb[h * SUB:(h + 1) * SUB]
                idx = sub + (u * TQ + t * GR + h * SUB)
                if top is None:
                    top = (val, idx, jnp.full((SUB, LANE), -jnp.inf, F32), idx)
                    continue
                m1, i1, m2, i2 = top
                g1 = val > m1
                g2 = val > m2
                top = (jnp.where(g1, val, m1), jnp.where(g1, idx, i1),
                       jnp.where(g1, m1, jnp.where(g2, val, m2)),
                       jnp.where(g1, i1, jnp.where(g2, idx, i2)))
        return top

    def select_tokens(top):
        vals = jnp.concatenate([top[0], top[2]], axis=0)
        ids = jnp.concatenate([top[1], top[3]], axis=0).astype(F32)
        big = float(S)
        m1 = jnp.max(vals)
        f1 = jnp.min(jnp.where(vals == m1, ids, big))
        vals2 = jnp.where(ids == f1, -jnp.inf, vals)
        m2 = jnp.max(vals2)
        f2 = jnp.min(jnp.where(jnp.logical_and(vals2 == m2, ids != f1), ids, big))
        i1 = jnp.minimum(f1.astype(jnp.int32), S - 1)
        i2 = jnp.minimum(f2.astype(jnp.int32), S - 1)
        idx_ref[0] = i1
        idx_ref[1] = i2
        sub = lax.broadcasted_iota(jnp.int32, (16, D), 0)

        def pick(ix):
            base = pl.multiple_of((ix // 16) * 16, 16)
            blk = xn_ref[pl.ds(base, 16), :].astype(F32)
            return jnp.sum(jnp.where(sub == ix - base, blk, 0.0), axis=0, keepdims=True)

        xs_ref[...] = jnp.where(sub == 0, pick(i1), jnp.where(sub == 1, pick(i2), 0.0)).astype(BF16)
        rs_ref[...] = jax.nn.sigmoid(jnp.where(sub == 0, m1, m2))

    def prep_k(slot):
        zz = jnp.zeros((PADW - DH, W), BF16)
        kp_ref[slot, 0] = jnp.concatenate([kt_buf[slot, 0], zz], axis=0).T
        kp_ref[slot, 1] = jnp.concatenate([zz, kt_buf[slot, 1]], axis=0).T

    def qproj_tile(u, n, slot):
        w = wq_buf[slot, :, n * LANE:(n + 1) * LANE]
        return (_nn(xn_ref[rows(u), :], w) * c).astype(BF16)

    def qproj_quarter(u, t, slot):
        return (_nn(xn_ref[rows(u, t, 4), :], wq_buf[slot]) * c).astype(BF16)

    def split_tiles(qv):
        return [qv[:, n * LANE:(n + 1) * LANE] for n in range(3)]

    def qk(q, h, slot):
        if isinstance(q, list):
            st = _nt(kp_ref[slot, h], jnp.concatenate(q[h:h + 2], axis=1))
        else:
            st = _nn(kp_ref[slot, h], q[h * LANE:h * LANE + PADW, :])
        s_refs[h][0] = st
        return jnp.max(st, axis=0, keepdims=True)

    def softmax(m, h):
        e = jnp.exp2(s_refs[h][z] - m)
        return e.astype(BF16), jnp.sum(e, axis=0, keepdims=True)

    def pv(p, l, h, slot, dep=None):
        one = 1.0 if dep is None else tie(dep[0:1, 0:1], 1.0)
        return (_nn(vt_buf[slot, h], p) * (one / l)).astype(BF16)

    def finish(u, val, n0, n1, part, nparts):
        r = rows(u, part, nparts)
        cs = slice(n0 * LANE, n1 * LANE)
        g = _silu(xg_ref[r, cs].astype(F32))
        out_buf[r, cs] = (x_buf[r, cs].astype(F32) + val * g).astype(out_buf.dtype)

    def finish_rows(u, chain):
        GR = 16
        for t in range(TQ // GR):
            r = pl.ds(u * TQ + t * GR, GR)
            gin = xg_ref[r, :].astype(F32)
            if len(chain) >= G_FIN:
                h = gin * tie(chain[-G_FIN], 0.5)
            else:
                h = gin * 0.5
            g = h + h * jnp.tanh(h)
            o = x_buf[r, :].astype(F32) + acc_ref[r, :] * g
            chain.append(o[:, D - 1:D])
            out_buf[r, :] = o.astype(out_buf.dtype)

    def wo_cols(u, o, slot, n0, n1, part=0, nparts=1, final=False):
        n = TQ // nparts
        r = rows(u, part, nparts)
        cs = slice(n0 * LANE, n1 * LANE)
        val = acc_ref[r, cs] + _nn(o[part * n:(part + 1) * n], wo_buf[slot, :, cs])
        if final:
            finish(u, val, n0, n1, part, nparts)
        else:
            acc_ref[r, cs] = val

    def unit(q, prev, bslot, a, cc, final=False, mid=None, dep0=None, dep1=None):
        m0 = qk(q, 0, bslot)
        m1 = qk(q, 1, bslot)
        if mid is not None:
            mid()
        p0 = softmax(m0, 0)
        p1 = softmax(m1, 1)
        o = prev.T
        if a is not None:
            qn = []
            for n in range(3):
                qn.append(qproj_tile(a[0], n, a[1]))
                wo_cols(cc[0], o, cc[1], n, n + 1, final=final)
            wo_cols(cc[0], o, cc[1], 3, 5, 0, 2, final=final)
            wo_cols(cc[0], o, cc[1], 3, 5, 1, 2, final=final)
        else:
            qn = None
            for t in range(4):
                wo_cols(cc[0], o, cc[1], 0, 5, t, 4, final=final)
        o0 = pv(*p0, 0, bslot, dep0)
        o1 = pv(*p1, 1, bslot, dep1)
        return qn, jnp.concatenate([o0, o1], axis=0)

    def load_carry():
        return q_st[...], ot_st[...]

    def store_carry(q, prev):
        q_st[...] = jnp.concatenate(q, axis=1).T
        ot_st[...] = prev

    def sync(starts=(), waits=()):
        def body(i, carry):
            for cp in starts:
                cp.start(priority=1)
            for cp in waits:
                cp.wait()
            return carry
        lax.fori_loop(0, z + 1, body, 0)

    def prologue():
        cp_wr = pltpu.make_async_copy(wr_hbm, wr_ref, sem_f.at[3])
        cp_wr.start()
        cp_x(0).start()
        cp_wq(0).start(priority=1)
        cp_k(0).start(priority=1)
        cp_x(1).start(priority=1)
        cp_v(0).start(priority=1)
        cp_x(0).wait()
        cp_wr.wait()
        top = layernorm(0, None)
        sync([cp_x(2), cp_wo(0), cp_x(3)], [cp_wq(0)])
        parts = [qproj_quarter(0, t, 0) for t in range(2)]
        sync([], [cp_k(0)])
        parts += [qproj_quarter(0, t, 0) for t in range(2, 4)]
        prep_k(0)
        q = split_tiles(jnp.concatenate(parts, axis=0))
        sync([cp_x(t) for t in range(4, U)] + [cp_k(1)], [cp_x(1)])
        top = layernorm(1, top, [])
        m0 = qk(q, 0, 0)
        m1 = qk(q, 1, 0)
        p0 = softmax(m0, 0)
        p1 = softmax(m1, 1)
        q = split_tiles(jnp.concatenate([qproj_quarter(1, t, 0) for t in range(4)], axis=0))
        plan = {1: [2], 2: [3, 4, 5], 3: [6, 7]}
        sync(list(cp_pair(1)) + [cp_k(2)], [cp_v(0), cp_wo(0), cp_x(2)])
        prev = jnp.concatenate([pv(*p0, 0, 0), pv(*p1, 1, 0)], axis=0)
        for u in range(1, R):
            if u == 2:
                sync(list(cp_pair(2)) + [cp_k(3)] + list(cp_ffn()), [cp_x(t) for t in range(3, U)] + [cp_k(1)])
            if u != 3:
                chain = []
            for t in plan[u]:
                top = layernorm(t, top, chain)
            q, prev = unit(q, prev, 0, (u + 1, 0), (u - 1, 0),
                           mid=(lambda: prep_k(1)) if u == R - 1 else None,
                           dep1=chain[-1] if u >= 2 else None)
        store_carry(q, prev)
        select_tokens(top)

    def ffn_block():
        for cp in cp_ffn():
            cp.wait()
        xs = xs_ref[...]
        gg = _nn(xs, wg_ref[...])
        uu = _nn(xs, wu_ref[...])
        hmid = (_silu(gg) * uu).astype(BF16)
        y = _nn(hmid, wd_ref[...]) * rs_ref[...]
        sub = lax.broadcasted_iota(jnp.int32, (16, D), 0)
        for k in range(2):
            ix = idx_ref[k]
            base = pl.multiple_of((ix // 16) * 16, 16)
            blk = xg_ref[pl.ds(base, 16), :].astype(F32)
            xg_ref[pl.ds(base, 16), :] = jnp.where(sub == ix - base, blk + y[k:k + 1, :], blk).astype(BF16)

    def main(j):
        s0 = slot_of(j)
        s1 = slot_of(j + 1)
        s2 = slot_of(j + 2)
        for cp in cp_pair(j + 1):
            cp.wait()

        @pl.when(j + 2 < NP)
        def _():
            cp_k(j + 2).wait()

        q, prev = load_carry()
        for v in range(U):
            u = (R + v) % U
            bs = s1 if v >= U - R else s0
            as_ = s1 if v + 1 >= U - R else s0
            cs_ = s1 if v - 1 >= U - R else s0
            mid = (lambda: prep_k(s2)) if v == U - 1 else None
            q, prev = unit(q, prev, bs, ((u + 1) % U, as_), ((u - 1) % U, cs_), mid=mid)
        store_carry(q, prev)

        @pl.when(j + 3 < NP)
        def _():
            for cp in cp_pair(j + 3):
                cp.start()

        @pl.when(j + 4 < NP)
        def _():
            cp_k(j + 4).start()

    def tail():
        p = slot_of(NP - 1)
        q, prev = load_carry()
        early = list(range(R - 1))

        def fence_out():
            return out_buf[pl.ds(pl.multiple_of(z * 16, 16), 16), 0:LANE].astype(F32)

        chain = []
        dep = None
        for u in range(R, U):
            a = (u + 1, p) if u + 1 < U else None
            if early:
                e = early.pop(0)
                finish_rows(e, chain)
                cp_out(e).start()
                dep = fence_out()
            q, prev = unit(q, prev, p, a, (u - 1, p), final=True, dep0=dep)
            cp_out(u - 1).start()
            dep = fence_out() if u + 1 < U else None
        o = prev.T
        for t in range(4):
            wo_cols(U - 1, o, p, 0, 5, t, 4, final=True)
            cp_out(U - 1, t, 4).start()
        for t in range(U - 1):
            cp_out(t).wait()
        for t in range(4):
            cp_out(U - 1, t, 4).wait()

    def everything():
        prologue()

        def loop_body(j, carry):
            pl.when(j == 1)(ffn_block)
            main(j)
            return carry
        lax.fori_loop(0, NP - 1, loop_body, 0)
        tail()

    pl.when(step == 0)(everything)


@jax.jit
def pallas_recurrent_scan__sliding_block_cached__moe_arch_mod__prompt_kernel(
        A_x, A_k_cache, A_v_cache, A_wq, A_wo, B_x, B_w_r, B_w_gate, B_w_up, B_w_down):
    B, S, D = A_x.shape
    _, H, SK, DH = A_k_cache.shape
    W = min(4096, max(256, SK // 4))
    NP = H // 2
    U = S // TQ
    FF = B_w_gate.shape[1]
    assert B == 1 and H % 2 == 0 and NP >= 4 and U == 8 and D == 5 * LANE and 2 * DH == 3 * LANE and W <= SK
    kern = functools.partial(_kernel, NP=NP, DH=DH, W=W, eps=1e-5)
    hbm = pl.BlockSpec(memory_space=pl.ANY)
    out = pl.pallas_call(
        kern,
        grid=(2,),
        in_specs=[hbm] * 9,
        out_specs=hbm,
        out_shape=jax.ShapeDtypeStruct((S, D), A_x.dtype),
        scratch_shapes=[
            pltpu.VMEM((S, D), BF16),
            pltpu.VMEM((S, D), BF16),
            pltpu.VMEM((S, D), BF16),
            pltpu.VMEM((S, D), F32),
            pltpu.VMEM((S, D), A_x.dtype),
            pltpu.VMEM((NSLOT, D, 2 * DH), BF16),
            pltpu.VMEM((NSLOT, 2 * DH, D), BF16),
            pltpu.VMEM((NSLOT, 2, DH, W), BF16),
            pltpu.VMEM((NSLOT, 2, DH, W), BF16),
            pltpu.VMEM((NSLOT, 2, W, 2 * LANE), BF16),
            pltpu.VMEM((2 * DH, TQ), BF16),
            pltpu.VMEM((2 * DH, TQ), BF16),
            pltpu.VMEM((1, W, TQ), F32),
            pltpu.VMEM((1, W, TQ), F32),
            pltpu.VMEM((16, D), BF16),
            pltpu.VMEM((16, D), F32),
            pltpu.SMEM((2,), jnp.int32),
            pltpu.VMEM((D,), BF16),
            pltpu.VMEM((D, FF), BF16),
            pltpu.VMEM((D, FF), BF16),
            pltpu.VMEM((FF, D), BF16),
            pltpu.SemaphoreType.DMA((U,)),
            pltpu.SemaphoreType.DMA((NSLOT,)),
            pltpu.SemaphoreType.DMA((NSLOT,)),
            pltpu.SemaphoreType.DMA((NSLOT,)),
            pltpu.SemaphoreType.DMA((NSLOT,)),
            pltpu.SemaphoreType.DMA((4,)),
            pltpu.SemaphoreType.DMA((U + 3,)),
        ],
        compiler_params=pltpu.CompilerParams(
            dimension_semantics=("arbitrary",),
            vmem_limit_bytes=100 * 1024 * 1024,
            disable_bounds_checks=True,
            disable_semaphore_checks=True),
        name="fused_attn_moe",
    )(A_x.reshape(S, D), jnp.swapaxes(A_k_cache, 2, 3), jnp.swapaxes(A_v_cache, 2, 3), A_wq, A_wo, B_w_r,
      B_w_gate, B_w_up, B_w_down)
    return out.reshape(B, S, D)
```

```python
import functools
import math

import jax
import jax.numpy as jnp
from jax import lax
import jax.experimental.pallas as pl
import jax.experimental.pallas.tpu as pltpu

F32 = jnp.float32
BF16 = jnp.bfloat16
LANE = 128
SUB = 8
NSLOT = 4
TQ = 256
R = 4
G_LN = 6
G_FIN = 3


def _nt(a, b):
    return lax.dot_general(a, b, (((1,), (1,)), ((), ())), preferred_element_type=F32)


def _nn(a, b):
    return jnp.dot(a, b, preferred_element_type=F32)


def _silu(x):
    h = 0.5 * x
    return h + h * jnp.tanh(h)


def _kernel(x_hbm, kt_hbm, vt_hbm, wq_hbm, wo_hbm, wr_hbm, wg_hbm, wu_hbm, wd_hbm,
            out_hbm,
            x_buf, xn_ref, xg_ref, acc_ref, out_buf, wq_buf, wo_buf, kt_buf, vt_buf, kp_ref,
            q_st, ot_st, s0_ref, s1_ref, xs_ref, rs_ref, idx_ref, wr_ref, wg_ref, wu_ref, wd_ref,
            sem_x, sem_wq, sem_wo, sem_k, sem_v, sem_f, sem_o,
            *, NP, DH, W, eps):
    S, D = x_buf.shape
    U = S // TQ
    PW = 2 * DH
    PADW = 2 * LANE
    SK = kt_hbm.shape[-1]
    c = (DH ** -0.5) * math.log2(math.e)
    step = pl.program_id(0)
    z = lax.shift_right_logical(step, 1)
    s_refs = (s0_ref, s1_ref)

    def slot_of(p):
        return p % NSLOT if isinstance(p, int) else p & (NSLOT - 1)

    def rows(u, part=0, nparts=1):
        n = TQ // nparts
        return pl.ds(u * TQ + part * n, n)

    def cp_x(t):
        return pltpu.make_async_copy(x_hbm.at[pl.ds(t * TQ, TQ)], x_buf.at[pl.ds(t * TQ, TQ)], sem_x.at[t])

    def col(p):
        return p * PW if isinstance(p, int) else pl.multiple_of(p * PW, LANE)

    def cp_wq(p):
        s = slot_of(p)
        return pltpu.make_async_copy(wq_hbm.at[:, pl.ds(col(p), PW)], wq_buf.at[s], sem_wq.at[s])

    def cp_wo(p):
        s = slot_of(p)
        return pltpu.make_async_copy(wo_hbm.at[pl.ds(col(p), PW)], wo_buf.at[s], sem_wo.at[s])

    def cp_k(p):
        s = slot_of(p)
        return pltpu.make_async_copy(kt_hbm.at[0, pl.ds(2 * p, 2), :, pl.ds(SK - W, W)], kt_buf.at[s], sem_k.at[s])

    def cp_v(p):
        s = slot_of(p)
        return pltpu.make_async_copy(vt_hbm.at[0, pl.ds(2 * p, 2), :, pl.ds(SK - W, W)], vt_buf.at[s], sem_v.at[s])

    def cp_pair(p):
        return (cp_wq(p), cp_v(p), cp_wo(p))

    def cp_ffn():
        return (pltpu.make_async_copy(wg_hbm, wg_ref, sem_f.at[0]),
                pltpu.make_async_copy(wu_hbm, wu_ref, sem_f.at[1]),
                pltpu.make_async_copy(wd_hbm, wd_ref, sem_f.at[2]))

    def cp_out(t, part=0, nparts=1):
        r = rows(t, part, nparts)
        return pltpu.make_async_copy(out_buf.at[r], out_hbm.at[r], sem_o.at[t + part])

    def tie(v, const):
        cb = lax.bitcast_convert_type(jnp.float32(const), jnp.int32)
        vb = lax.bitcast_convert_type(v, jnp.int32)
        return lax.bitcast_convert_type(jnp.minimum((vb & 0x7FFFFFFF) | cb, cb), F32)

    def layernorm(u, top, chain=None):
        GR = 16
        wr = wr_ref[...].astype(F32).reshape(1, D)
        sub = lax.broadcasted_iota(jnp.int32, (SUB, LANE), 0)
        for t in range(TQ // GR):
            r = pl.ds(u * TQ + t * GR, GR)
            x = x_buf[r, :].astype(F32)
            ssum = jnp.sum(x, axis=-1, keepdims=True)
            if chain is not None and len(chain) >= G_LN:
                m = ssum * tie(chain[-G_LN], 1.0 / D)
            else:
                m = ssum * (1.0 / D)
            xc = x - m
            v = jnp.sum(xc * xc, axis=-1, keepdims=True) * (1.0 / D)
            xf = xc * lax.rsqrt(v + eps)
            xn = xf.astype(BF16)
            xn_ref[r, :] = xn
            xg_ref[r, :] = xn
            sc = jnp.sum(xf * wr, axis=-1, keepdims=True)
            sc = sc.astype(BF16).astype(F32)
            if chain is not None:
                chain.append(sc)
            scb = jnp.broadcast_to(sc, (GR, LANE))
            for h in range(GR // SUB):
                val = scb[h * SUB:(h + 1) * SUB]
                idx = sub + (u * TQ + t * GR + h * SUB)
                if top is None:
                    top = (val, idx, jnp.full((SUB, LANE), -jnp.inf, F32), idx)
                    continue
                m1, i1, m2, i2 = top
                g1 = val > m1
                g2 = val > m2
                top = (jnp.where(g1, val, m1), jnp.where(g1, idx, i1),
                       jnp.where(g1, m1, jnp.where(g2, val, m2)),
                       jnp.where(g1, i1, jnp.where(g2, idx, i2)))
        return top

    def select_tokens(top):
        vals = jnp.concatenate([top[0], top[2]], axis=0)
        ids = jnp.concatenate([top[1], top[3]], axis=0).astype(F32)
        big = float(S)
        m1 = jnp.max(vals)
        f1 = jnp.min(jnp.where(vals == m1, ids, big))
        vals2 = jnp.where(ids == f1, -jnp.inf, vals)
        m2 = jnp.max(vals2)
        f2 = jnp.min(jnp.where(jnp.logical_and(vals2 == m2, ids != f1), ids, big))
        i1 = jnp.minimum(f1.astype(jnp.int32), S - 1)
        i2 = jnp.minimum(f2.astype(jnp.int32), S - 1)
        idx_ref[0] = i1
        idx_ref[1] = i2
        sub = lax.broadcasted_iota(jnp.int32, (16, D), 0)

        def pick(ix):
            base = pl.multiple_of((ix // 16) * 16, 16)
            blk = xn_ref[pl.ds(base, 16), :].astype(F32)
            return jnp.sum(jnp.where(sub == ix - base, blk, 0.0), axis=0, keepdims=True)

        xs_ref[...] = jnp.where(sub == 0, pick(i1), jnp.where(sub == 1, pick(i2), 0.0)).astype(BF16)
        rs_ref[...] = jax.nn.sigmoid(jnp.where(sub == 0, m1, m2))

    def prep_k(slot):
        zz = jnp.zeros((PADW - DH, W), BF16)
        kp_ref[slot, 0] = jnp.concatenate([kt_buf[slot, 0], zz], axis=0).T
        kp_ref[slot, 1] = jnp.concatenate([zz, kt_buf[slot, 1]], axis=0).T

    def qproj_tile(u, n, slot):
        w = wq_buf[slot, :, n * LANE:(n + 1) * LANE]
        return (_nn(xn_ref[rows(u), :], w) * c).astype(BF16)

    def qproj_quarter(u, t, slot):
        return (_nn(xn_ref[rows(u, t, 4), :], wq_buf[slot]) * c).astype(BF16)

    def split_tiles(qv):
        return [qv[:, n * LANE:(n + 1) * LANE] for n in range(3)]

    def qk(q, h, slot):
        if isinstance(q, list):
            st = _nt(kp_ref[slot, h], jnp.concatenate(q[h:h + 2], axis=1))
        else:
            st = _nn(kp_ref[slot, h], q[h * LANE:h * LANE + PADW, :])
        s_refs[h][0] = st
        return jnp.max(st, axis=0, keepdims=True)

    def softmax(m, h):
        e = jnp.exp2(s_refs[h][z] - m)
        return e.astype(BF16), jnp.sum(e, axis=0, keepdims=True)

    def pv(p, l, h, slot, dep=None):
        one = 1.0 if dep is None else tie(dep[0:1, 0:1], 1.0)
        return (_nn(vt_buf[slot, h], p) * (one / l)).astype(BF16)

    def finish(u, val, n0, n1, part, nparts):
        r = rows(u, part, nparts)
        cs = slice(n0 * LANE, n1 * LANE)
        g = _silu(xg_ref[r, cs].astype(F32))
        out_buf[r, cs] = (x_buf[r, cs].astype(F32) + val * g).astype(out_buf.dtype)

    def finish_rows(u, chain):
        GR = 16
        for t in range(TQ // GR):
            r = pl.ds(u * TQ + t * GR, GR)
            gin = xg_ref[r, :].astype(F32)
            if len(chain) >= G_FIN:
                h = gin * tie(chain[-G_FIN], 0.5)
            else:
                h = gin * 0.5
            g = h + h * jnp.tanh(h)
            o = x_buf[r, :].astype(F32) + acc_ref[r, :] * g
            chain.append(o[:, D - 1:D])
            out_buf[r, :] = o.astype(out_buf.dtype)

    def wo_cols(u, o, slot, n0, n1, part=0, nparts=1, final=False, init=False):
        n = TQ // nparts
        r = rows(u, part, nparts)
        cs = slice(n0 * LANE, n1 * LANE)
        if init:
            val = _nn(o[part * n:(part + 1) * n], wo_buf[slot, :, cs])
        else:
            val = acc_ref[r, cs] + _nn(o[part * n:(part + 1) * n], wo_buf[slot, :, cs])
        if final:
            finish(u, val, n0, n1, part, nparts)
        else:
            acc_ref[r, cs] = val

    def unit(q, prev, bslot, a, cc, final=False, init=False, mid=None, dep0=None, dep1=None):
        m0 = qk(q, 0, bslot)
        m1 = qk(q, 1, bslot)
        if mid is not None:
            mid()
        p0 = softmax(m0, 0)
        p1 = softmax(m1, 1)
        o = prev.T
        if a is not None:
            qn = []
            for n in range(3):
                qn.append(qproj_tile(a[0], n, a[1]))
                wo_cols(cc[0], o, cc[1], n, n + 1, final=final, init=init)
            wo_cols(cc[0], o, cc[1], 3, 5, 0, 2, final=final, init=init)
            wo_cols(cc[0], o, cc[1], 3, 5, 1, 2, final=final, init=init)
        else:
            qn = None
            for t in range(4):
                wo_cols(cc[0], o, cc[1], 0, 5, t, 4, final=final)
        o0 = pv(*p0, 0, bslot, dep0)
        o1 = pv(*p1, 1, bslot, dep1)
        return qn, jnp.concatenate([o0, o1], axis=0)

    def load_carry():
        return q_st[...], ot_st[...]

    def store_carry(q, prev):
        q_st[...] = jnp.concatenate(q, axis=1).T
        ot_st[...] = prev

    def sync(starts=(), waits=()):
        def body(i, carry):
            for cp in starts:
                cp.start(priority=1)
            for cp in waits:
                cp.wait()
            return carry
        lax.fori_loop(0, z + 1, body, 0)

    def prologue():
        cp_wr = pltpu.make_async_copy(wr_hbm, wr_ref, sem_f.at[3])
        cp_wr.start()
        cp_x(0).start()
        cp_wq(0).start(priority=1)
        cp_k(0).start(priority=1)
        cp_x(1).start(priority=1)
        cp_v(0).start(priority=1)
        acc_ref[pl.ds((R - 1) * TQ, S - (R - 1) * TQ), :] = jnp.zeros((S - (R - 1) * TQ, D), F32)
        cp_x(0).wait()
        cp_wr.wait()
        top = layernorm(0, None)
        sync([cp_x(2), cp_wo(0), cp_x(3)], [cp_wq(0)])
        parts = [qproj_quarter(0, t, 0) for t in range(2)]
        sync([], [cp_k(0)])
        parts += [qproj_quarter(0, t, 0) for t in range(2, 4)]
        prep_k(0)
        q = split_tiles(jnp.concatenate(parts, axis=0))
        sync([cp_x(t) for t in range(4, U)] + [cp_k(1)], [cp_x(1)])
        top = layernorm(1, top, [])
        m0 = qk(q, 0, 0)
        m1 = qk(q, 1, 0)
        p0 = softmax(m0, 0)
        p1 = softmax(m1, 1)
        q = split_tiles(jnp.concatenate([qproj_quarter(1, t, 0) for t in range(4)], axis=0))
        plan = {1: [2], 2: [3, 4, 5], 3: [6, 7]}
        sync(list(cp_pair(1)) + [cp_k(2)], [cp_v(0), cp_wo(0), cp_x(2)])
        prev = jnp.concatenate([pv(*p0, 0, 0), pv(*p1, 1, 0)], axis=0)
        for u in range(1, R):
            if u == 2:
                sync(list(cp_pair(2)) + [cp_k(3)] + list(cp_ffn()), [cp_x(t) for t in range(3, U)] + [cp_k(1)])
            if u != 3:
                chain = []
            for t in plan[u]:
                top = layernorm(t, top, chain)
            q, prev = unit(q, prev, 0, (u + 1, 0), (u - 1, 0), init=True,
                           mid=(lambda: prep_k(1)) if u == R - 1 else None,
                           dep1=chain[-1] if u >= 2 else None)
        store_carry(q, prev)
        select_tokens(top)

    def ffn_block():
        for cp in cp_ffn():
            cp.wait()
        xs = xs_ref[...]
        gg = _nn(xs, wg_ref[...])
        uu = _nn(xs, wu_ref[...])
        hmid = (_silu(gg) * uu).astype(BF16)
        y = _nn(hmid, wd_ref[...]) * rs_ref[...]
        sub = lax.broadcasted_iota(jnp.int32, (16, D), 0)
        for k in range(2):
            ix = idx_ref[k]
            base = pl.multiple_of((ix // 16) * 16, 16)
            blk = xg_ref[pl.ds(base, 16), :].astype(F32)
            xg_ref[pl.ds(base, 16), :] = jnp.where(sub == ix - base, blk + y[k:k + 1, :], blk).astype(BF16)

    def main(j):
        s0 = slot_of(j)
        s1 = slot_of(j + 1)
        s2 = slot_of(j + 2)
        for cp in cp_pair(j + 1):
            cp.wait()

        @pl.when(j + 2 < NP)
        def _():
            cp_k(j + 2).wait()

        q, prev = load_carry()
        for v in range(U):
            u = (R + v) % U
            bs = s1 if v >= U - R else s0
            as_ = s1 if v + 1 >= U - R else s0
            cs_ = s1 if v - 1 >= U - R else s0
            mid = (lambda: prep_k(s2)) if v == U - 1 else None
            q, prev = unit(q, prev, bs, ((u + 1) % U, as_), ((u - 1) % U, cs_), mid=mid)
        store_carry(q, prev)

        @pl.when(j + 3 < NP)
        def _():
            for cp in cp_pair(j + 3):
                cp.start()

        @pl.when(j + 4 < NP)
        def _():
            cp_k(j + 4).start()

    def tail():
        p = slot_of(NP - 1)
        q, prev = load_carry()
        early = list(range(R - 1))

        def fence_out():
            return out_buf[pl.ds(pl.multiple_of(z * 16, 16), 16), 0:LANE].astype(F32)

        chain = []
        dep = None
        for u in range(R, U):
            a = (u + 1, p) if u + 1 < U else None
            if early:
                e = early.pop(0)
                finish_rows(e, chain)
                cp_out(e).start()
                dep = fence_out()
            q, prev = unit(q, prev, p, a, (u - 1, p), final=True, dep0=dep)
            cp_out(u - 1).start()
            dep = fence_out() if u + 1 < U else None
        o = prev.T
        for t in range(4):
            wo_cols(U - 1, o, p, 0, 5, t, 4, final=True)
            cp_out(U - 1, t, 4).start()
        for t in range(U - 1):
            cp_out(t).wait()
        for t in range(4):
            cp_out(U - 1, t, 4).wait()

    def everything():
        prologue()

        def loop_body(j, carry):
            pl.when(j == 1)(ffn_block)
            main(j)
            return carry
        lax.fori_loop(0, NP - 1, loop_body, 0)
        tail()

    pl.when(step == 0)(everything)


@jax.jit
def pallas_recurrent_scan__sliding_block_cached__moe_arch_mod__prompt_kernel(
        A_x, A_k_cache, A_v_cache, A_wq, A_wo, B_x, B_w_r, B_w_gate, B_w_up, B_w_down):
    B, S, D = A_x.shape
    _, H, SK, DH = A_k_cache.shape
    W = min(4096, max(256, SK // 4))
    NP = H // 2
    U = S // TQ
    FF = B_w_gate.shape[1]
    assert B == 1 and H % 2 == 0 and NP >= 4 and U == 8 and D == 5 * LANE and 2 * DH == 3 * LANE and W <= SK
    kern = functools.partial(_kernel, NP=NP, DH=DH, W=W, eps=1e-5)
    hbm = pl.BlockSpec(memory_space=pl.ANY)
    out = pl.pallas_call(
        kern,
        grid=(2,),
        in_specs=[hbm] * 9,
        out_specs=hbm,
        out_shape=jax.ShapeDtypeStruct((S, D), A_x.dtype),
        scratch_shapes=[
            pltpu.VMEM((S, D), BF16),
            pltpu.VMEM((S, D), BF16),
            pltpu.VMEM((S, D), BF16),
            pltpu.VMEM((S, D), F32),
            pltpu.VMEM((S, D), A_x.dtype),
            pltpu.VMEM((NSLOT, D, 2 * DH), BF16),
            pltpu.VMEM((NSLOT, 2 * DH, D), BF16),
            pltpu.VMEM((NSLOT, 2, DH, W), BF16),
            pltpu.VMEM((NSLOT, 2, DH, W), BF16),
            pltpu.VMEM((NSLOT, 2, W, 2 * LANE), BF16),
            pltpu.VMEM((2 * DH, TQ), BF16),
            pltpu.VMEM((2 * DH, TQ), BF16),
            pltpu.VMEM((1, W, TQ), F32),
            pltpu.VMEM((1, W, TQ), F32),
            pltpu.VMEM((16, D), BF16),
            pltpu.VMEM((16, D), F32),
            pltpu.SMEM((2,), jnp.int32),
            pltpu.VMEM((D,), BF16),
            pltpu.VMEM((D, FF), BF16),
            pltpu.VMEM((D, FF), BF16),
            pltpu.VMEM((FF, D), BF16),
            pltpu.SemaphoreType.DMA((U,)),
            pltpu.SemaphoreType.DMA((NSLOT,)),
            pltpu.SemaphoreType.DMA((NSLOT,)),
            pltpu.SemaphoreType.DMA((NSLOT,)),
            pltpu.SemaphoreType.DMA((NSLOT,)),
            pltpu.SemaphoreType.DMA((4,)),
            pltpu.SemaphoreType.DMA((U + 3,)),
        ],
        compiler_params=pltpu.CompilerParams(
            dimension_semantics=("arbitrary",),
            vmem_limit_bytes=100 * 1024 * 1024,
            disable_bounds_checks=True,
            disable_semaphore_checks=True),
        name="fused_attn_moe",
    )(A_x.reshape(S, D), jnp.swapaxes(A_k_cache, 2, 3), jnp.swapaxes(A_v_cache, 2, 3), A_wq, A_wo, B_w_r,
      B_w_gate, B_w_up, B_w_down)
    return out.reshape(B, S, D)
```

```python
import functools
import math

import jax
import jax.numpy as jnp
from jax import lax
import jax.experimental.pallas as pl
import jax.experimental.pallas.tpu as pltpu

F32 = jnp.float32
BF16 = jnp.bfloat16
LANE = 128
SUB = 8
NSLOT = 4
TQ = 256
R = 4
G_LN = 6
G_FIN = 3


def _nt(a, b):
    return lax.dot_general(a, b, (((1,), (1,)), ((), ())), preferred_element_type=F32)


def _nn(a, b):
    return jnp.dot(a, b, preferred_element_type=F32)


def _silu(x):
    h = 0.5 * x
    return h + h * jnp.tanh(h)


def _kernel(x_hbm, kt_hbm, vt_hbm, wq_hbm, wo_hbm, wr_hbm, wg_hbm, wu_hbm, wd_hbm,
            out_hbm,
            x_buf, xn_ref, xg_ref, acc_ref, out_buf, wq_buf, wo_buf, kt_buf, vt_buf, kp_ref,
            q_st, ot_st, p_st, s0_ref, s1_ref, xs_ref, rs_ref, idx_ref, wr_ref, wg_ref, wu_ref, wd_ref,
            sem_x, sem_wq, sem_wo, sem_k, sem_v, sem_f, sem_o,
            *, NP, DH, W, eps):
    S, D = x_buf.shape
    U = S // TQ
    PW = 2 * DH
    PADW = 2 * LANE
    SK = kt_hbm.shape[-1]
    c = (DH ** -0.5) * math.log2(math.e)
    step = pl.program_id(0)
    z = lax.shift_right_logical(step, 1)
    s_refs = (s0_ref, s1_ref)

    def slot_of(p):
        return p % NSLOT if isinstance(p, int) else p & (NSLOT - 1)

    def rows(u, part=0, nparts=1):
        n = TQ // nparts
        return pl.ds(u * TQ + part * n, n)

    def cp_x(t):
        return pltpu.make_async_copy(x_hbm.at[pl.ds(t * TQ, TQ)], x_buf.at[pl.ds(t * TQ, TQ)], sem_x.at[t])

    def col(p):
        return p * PW if isinstance(p, int) else pl.multiple_of(p * PW, LANE)

    def cp_wq(p):
        s = slot_of(p)
        return pltpu.make_async_copy(wq_hbm.at[:, pl.ds(col(p), PW)], wq_buf.at[s], sem_wq.at[s])

    def cp_wo(p):
        s = slot_of(p)
        return pltpu.make_async_copy(wo_hbm.at[pl.ds(col(p), PW)], wo_buf.at[s], sem_wo.at[s])

    def cp_k(p):
        s = slot_of(p)
        return pltpu.make_async_copy(kt_hbm.at[0, pl.ds(2 * p, 2), :, pl.ds(SK - W, W)], kt_buf.at[s], sem_k.at[s])

    def cp_v(p):
        s = slot_of(p)
        return pltpu.make_async_copy(vt_hbm.at[0, pl.ds(2 * p, 2), :, pl.ds(SK - W, W)], vt_buf.at[s], sem_v.at[s])

    def cp_pair(p):
        return (cp_wq(p), cp_v(p), cp_wo(p))

    def cp_ffn():
        return (pltpu.make_async_copy(wg_hbm, wg_ref, sem_f.at[0]),
                pltpu.make_async_copy(wu_hbm, wu_ref, sem_f.at[1]),
                pltpu.make_async_copy(wd_hbm, wd_ref, sem_f.at[2]))

    def cp_out(t, part=0, nparts=1):
        r = rows(t, part, nparts)
        return pltpu.make_async_copy(out_buf.at[r], out_hbm.at[r], sem_o.at[t + part])

    def tie(v, const):
        cb = lax.bitcast_convert_type(jnp.float32(const), jnp.int32)
        vb = lax.bitcast_convert_type(v, jnp.int32)
        return lax.bitcast_convert_type(jnp.minimum((vb & 0x7FFFFFFF) | cb, cb), F32)

    def layernorm(u, top, chain=None):
        GR = 16
        wr = wr_ref[...].astype(F32).reshape(1, D)
        sub = lax.broadcasted_iota(jnp.int32, (SUB, LANE), 0)
        for t in range(TQ // GR):
            r = pl.ds(u * TQ + t * GR, GR)
            x = x_buf[r, :].astype(F32)
            ssum = jnp.sum(x, axis=-1, keepdims=True)
            if chain is not None and len(chain) >= G_LN:
                m = ssum * tie(chain[-G_LN], 1.0 / D)
            else:
                m = ssum * (1.0 / D)
            xc = x - m
            v = jnp.sum(xc * xc, axis=-1, keepdims=True) * (1.0 / D)
            xf = xc * lax.rsqrt(v + eps)
            xn = xf.astype(BF16)
            xn_ref[r, :] = xn
            xg_ref[r, :] = xn
            sc = jnp.sum(xf * wr, axis=-1, keepdims=True)
            sc = sc.astype(BF16).astype(F32)
            if chain is not None:
                chain.append(sc)
            scb = jnp.broadcast_to(sc, (GR, LANE))
            for h in range(GR // SUB):
                val = scb[h * SUB:(h + 1) * SUB]
                idx = sub + (u * TQ + t * GR + h * SUB)
                if top is None:
                    top = (val, idx, jnp.full((SUB, LANE), -jnp.inf, F32), idx)
                    continue
                m1, i1, m2, i2 = top
                g1 = val > m1
                g2 = val > m2
                top = (jnp.where(g1, val, m1), jnp.where(g1, idx, i1),
                       jnp.where(g1, m1, jnp.where(g2, val, m2)),
                       jnp.where(g1, i1, jnp.where(g2, idx, i2)))
        return top

    def select_tokens(top):
        vals = jnp.concatenate([top[0], top[2]], axis=0)
        ids = jnp.concatenate([top[1], top[3]], axis=0).astype(F32)
        big = float(S)
        m1 = jnp.max(vals)
        f1 = jnp.min(jnp.where(vals == m1, ids, big))
        vals2 = jnp.where(ids == f1, -jnp.inf, vals)
        m2 = jnp.max(vals2)
        f2 = jnp.min(jnp.where(jnp.logical_and(vals2 == m2, ids != f1), ids, big))
        i1 = jnp.minimum(f1.astype(jnp.int32), S - 1)
        i2 = jnp.minimum(f2.astype(jnp.int32), S - 1)
        idx_ref[0] = i1
        idx_ref[1] = i2
        sub = lax.broadcasted_iota(jnp.int32, (16, D), 0)

        def pick(ix):
            base = pl.multiple_of((ix // 16) * 16, 16)
            blk = xn_ref[pl.ds(base, 16), :].astype(F32)
            return jnp.sum(jnp.where(sub == ix - base, blk, 0.0), axis=0, keepdims=True)

        xs_ref[...] = jnp.where(sub == 0, pick(i1), jnp.where(sub == 1, pick(i2), 0.0)).astype(BF16)
        rs_ref[...] = jax.nn.sigmoid(jnp.where(sub == 0, m1, m2))

    def prep_k(slot):
        zz = jnp.zeros((PADW - DH, W), BF16)
        kp_ref[slot, 0] = jnp.concatenate([kt_buf[slot, 0], zz], axis=0).T
        kp_ref[slot, 1] = jnp.concatenate([zz, kt_buf[slot, 1]], axis=0).T

    def qproj_tile(u, n, slot):
        w = wq_buf[slot, :, n * LANE:(n + 1) * LANE]
        return (_nn(xn_ref[rows(u), :], w) * c).astype(BF16)

    def qproj_quarter(u, t, slot):
        return (_nn(xn_ref[rows(u, t, 4), :], wq_buf[slot]) * c).astype(BF16)

    def split_tiles(qv):
        return [qv[:, n * LANE:(n + 1) * LANE] for n in range(3)]

    def qk(q, h, slot):
        if isinstance(q, list):
            st = _nt(kp_ref[slot, h], jnp.concatenate(q[h:h + 2], axis=1))
        else:
            st = _nn(kp_ref[slot, h], q[h * LANE:h * LANE + PADW, :])
        s_refs[h][0] = st
        return jnp.max(st, axis=0, keepdims=True)

    def softmax(m, h):
        e = jnp.exp2(s_refs[h][z] - m)
        return e.astype(BF16), jnp.sum(e, axis=0, keepdims=True)

    def pv(p, l, h, slot, dep=None):
        one = 1.0 if dep is None else tie(dep[0:1, 0:1], 1.0)
        return (_nn(vt_buf[slot, h], p) * (one / l)).astype(BF16)

    def finish(u, val, n0, n1, part, nparts):
        r = rows(u, part, nparts)
        cs = slice(n0 * LANE, n1 * LANE)
        g = _silu(xg_ref[r, cs].astype(F32))
        out_buf[r, cs] = (x_buf[r, cs].astype(F32) + val * g).astype(out_buf.dtype)

    def finish_rows(u, chain):
        GR = 16
        for t in range(TQ // GR):
            r = pl.ds(u * TQ + t * GR, GR)
            gin = xg_ref[r, :].astype(F32)
            if len(chain) >= G_FIN:
                h = gin * tie(chain[-G_FIN], 0.5)
            else:
                h = gin * 0.5
            g = h + h * jnp.tanh(h)
            o = x_buf[r, :].astype(F32) + acc_ref[r, :] * g
            chain.append(o[:, D - 1:D])
            out_buf[r, :] = o.astype(out_buf.dtype)

    def wo_cols(u, o, slot, n0, n1, part=0, nparts=1, final=False, init=False):
        n = TQ // nparts
        r = rows(u, part, nparts)
        cs = slice(n0 * LANE, n1 * LANE)
        if init:
            val = _nn(o[part * n:(part + 1) * n], wo_buf[slot, :, cs])
        else:
            val = acc_ref[r, cs] + _nn(o[part * n:(part + 1) * n], wo_buf[slot, :, cs])
        if final:
            finish(u, val, n0, n1, part, nparts)
        else:
            acc_ref[r, cs] = val

    def unit(q, prev, bslot, a, cc, final=False, init=False, mid=None, dep0=None, dep1=None):
        m0 = qk(q, 0, bslot)
        m1 = qk(q, 1, bslot)
        if mid is not None:
            mid()
        p0 = softmax(m0, 0)
        p1 = softmax(m1, 1)
        o = prev.T
        if a is not None:
            qn = []
            for n in range(3):
                qn.append(qproj_tile(a[0], n, a[1]))
                wo_cols(cc[0], o, cc[1], n, n + 1, final=final, init=init)
            wo_cols(cc[0], o, cc[1], 3, 5, 0, 2, final=final, init=init)
            wo_cols(cc[0], o, cc[1], 3, 5, 1, 2, final=final, init=init)
        else:
            qn = None
            for t in range(2):
                wo_cols(cc[0], o, cc[1], 0, 5, t, 4, final=final)
        o0 = pv(*p0, 0, bslot, dep0)
        o1 = pv(*p1, 1, bslot, dep1)
        if a is None:
            for t in range(2, 4):
                wo_cols(cc[0], o, cc[1], 0, 5, t, 4, final=final)
        return qn, jnp.concatenate([o0, o1], axis=0)

    def load_carry():
        return q_st[...], ot_st[...]

    def store_carry(q, prev):
        q_st[...] = jnp.concatenate(q, axis=1).T
        ot_st[...] = prev

    def sync(starts=(), waits=()):
        def body(i, carry):
            for cp in starts:
                cp.start(priority=1)
            for cp in waits:
                cp.wait()
            return carry
        lax.fori_loop(0, z + 1, body, 0)

    def prologue():
        cp_wr = pltpu.make_async_copy(wr_hbm, wr_ref, sem_f.at[3])
        cp_wr.start()
        cp_x(0).start()
        cp_wq(0).start(priority=1)
        cp_k(0).start(priority=1)
        cp_x(1).start(priority=1)
        cp_v(0).start(priority=1)
        acc_ref[pl.ds((R - 1) * TQ, S - (R - 1) * TQ), :] = jnp.zeros((S - (R - 1) * TQ, D), F32)
        cp_x(0).wait()
        cp_wr.wait()
        top = layernorm(0, None)
        sync([cp_x(2), cp_wo(0), cp_x(3)], [cp_wq(0)])
        parts = [qproj_quarter(0, t, 0) for t in range(2)]
        sync([], [cp_k(0)])
        parts += [qproj_quarter(0, t, 0) for t in range(2, 4)]
        prep_k(0)
        q = split_tiles(jnp.concatenate(parts, axis=0))
        sync([cp_x(t) for t in range(4, U)] + [cp_k(1)], [cp_x(1)])
        top = layernorm(1, top, [])
        m0 = qk(q, 0, 0)
        m1 = qk(q, 1, 0)
        ls = []
        for h, m in enumerate((m0, m1)):
            l8 = None
            for i in range(W // 16):
                e = jnp.exp2(s_refs[h][z, 16 * i:16 * i + 16, :] - m)
                p_st[h, 16 * i:16 * i + 16, :] = e.astype(BF16)
                e8 = e[0:8] + e[8:16]
                l8 = e8 if l8 is None else l8 + e8
            ls.append(jnp.sum(l8, axis=0, keepdims=True))
        q = split_tiles(jnp.concatenate([qproj_quarter(1, t, 0) for t in range(4)], axis=0))
        plan = {1: [2], 2: [3, 4, 5], 3: [6, 7]}
        sync(list(cp_pair(1)) + [cp_k(2)], [cp_v(0), cp_wo(0), cp_x(2)])
        prev = jnp.concatenate([pv(p_st[0], ls[0], 0, 0), pv(p_st[1], ls[1], 1, 0)], axis=0)
        for u in range(1, R):
            if u == 2:
                sync(list(cp_pair(2)) + [cp_k(3)] + list(cp_ffn()), [cp_x(t) for t in range(3, U)] + [cp_k(1)])
            if u != 3:
                chain = []
            for t in plan[u]:
                top = layernorm(t, top, chain)
            q, prev = unit(q, prev, 0, (u + 1, 0), (u - 1, 0), init=True,
                           mid=(lambda: prep_k(1)) if u == R - 1 else None,
                           dep1=chain[-1] if u >= 2 else None)
        store_carry(q, prev)
        select_tokens(top)

    def ffn_block():
        for cp in cp_ffn():
            cp.wait()
        xs = xs_ref[...]
        gg = _nn(xs, wg_ref[...])
        uu = _nn(xs, wu_ref[...])
        hmid = (_silu(gg) * uu).astype(BF16)
        y = _nn(hmid, wd_ref[...]) * rs_ref[...]
        sub = lax.broadcasted_iota(jnp.int32, (16, D), 0)
        for k in range(2):
            ix = idx_ref[k]
            base = pl.multiple_of((ix // 16) * 16, 16)
            blk = xg_ref[pl.ds(base, 16), :].astype(F32)
            xg_ref[pl.ds(base, 16), :] = jnp.where(sub == ix - base, blk + y[k:k + 1, :], blk).astype(BF16)

    def main(j):
        s0 = slot_of(j)
        s1 = slot_of(j + 1)
        s2 = slot_of(j + 2)
        for cp in cp_pair(j + 1):
            cp.wait()

        @pl.when(j + 2 < NP)
        def _():
            cp_k(j + 2).wait()

        q, prev = load_carry()
        for v in range(U):
            u = (R + v) % U
            bs = s1 if v >= U - R else s0
            as_ = s1 if v + 1 >= U - R else s0
            cs_ = s1 if v - 1 >= U - R else s0
            mid = (lambda: prep_k(s2)) if v == U - 1 else None
            q, prev = unit(q, prev, bs, ((u + 1) % U, as_), ((u - 1) % U, cs_), mid=mid)
        store_carry(q, prev)

        @pl.when(j + 3 < NP)
        def _():
            for cp in cp_pair(j + 3):
                cp.start()

        @pl.when(j + 4 < NP)
        def _():
            cp_k(j + 4).start()

    def tail():
        p = slot_of(NP - 1)
        q, prev = load_carry()
        early = list(range(R - 1))

        def fence_out():
            return out_buf[pl.ds(pl.multiple_of(z * 16, 16), 16), 0:LANE].astype(F32)

        chain = []
        dep = None
        for u in range(R, U):
            a = (u + 1, p) if u + 1 < U else None
            if early:
                e = early.pop(0)
                finish_rows(e, chain)
                cp_out(e).start()
                dep = fence_out()
            q, prev = unit(q, prev, p, a, (u - 1, p), final=True, dep0=dep)
            cp_out(u - 1).start()
            dep = fence_out() if u + 1 < U else None
        o = prev.T
        for t in range(4):
            wo_cols(U - 1, o, p, 0, 5, t, 4, final=True)
            cp_out(U - 1, t, 4).start()
        for t in range(U - 1):
            cp_out(t).wait()
        for t in range(4):
            cp_out(U - 1, t, 4).wait()

    def everything():
        prologue()

        def loop_body(j, carry):
            main(j)
            return carry
        lax.fori_loop(0, NP - 1, loop_body, 0)
        ffn_block()
        tail()

    pl.when(step == 0)(everything)


@jax.jit
def pallas_recurrent_scan__sliding_block_cached__moe_arch_mod__prompt_kernel(
        A_x, A_k_cache, A_v_cache, A_wq, A_wo, B_x, B_w_r, B_w_gate, B_w_up, B_w_down):
    B, S, D = A_x.shape
    _, H, SK, DH = A_k_cache.shape
    W = min(4096, max(256, SK // 4))
    NP = H // 2
    U = S // TQ
    FF = B_w_gate.shape[1]
    assert B == 1 and H % 2 == 0 and NP >= 4 and U == 8 and D == 5 * LANE and 2 * DH == 3 * LANE and W <= SK
    kern = functools.partial(_kernel, NP=NP, DH=DH, W=W, eps=1e-5)
    hbm = pl.BlockSpec(memory_space=pl.ANY)
    out = pl.pallas_call(
        kern,
        grid=(2,),
        in_specs=[hbm] * 9,
        out_specs=hbm,
        out_shape=jax.ShapeDtypeStruct((S, D), A_x.dtype),
        scratch_shapes=[
            pltpu.VMEM((S, D), BF16),
            pltpu.VMEM((S, D), BF16),
            pltpu.VMEM((S, D), BF16),
            pltpu.VMEM((S, D), F32),
            pltpu.VMEM((S, D), A_x.dtype),
            pltpu.VMEM((NSLOT, D, 2 * DH), BF16),
            pltpu.VMEM((NSLOT, 2 * DH, D), BF16),
            pltpu.VMEM((NSLOT, 2, DH, W), BF16),
            pltpu.VMEM((NSLOT, 2, DH, W), BF16),
            pltpu.VMEM((NSLOT, 2, W, 2 * LANE), BF16),
            pltpu.VMEM((2 * DH, TQ), BF16),
            pltpu.VMEM((2 * DH, TQ), BF16),
            pltpu.VMEM((2, W, TQ), BF16),
            pltpu.VMEM((1, W, TQ), F32),
            pltpu.VMEM((1, W, TQ), F32),
            pltpu.VMEM((16, D), BF16),
            pltpu.VMEM((16, D), F32),
            pltpu.SMEM((2,), jnp.int32),
            pltpu.VMEM((D,), BF16),
            pltpu.VMEM((D, FF), BF16),
            pltpu.VMEM((D, FF), BF16),
            pltpu.VMEM((FF, D), BF16),
            pltpu.SemaphoreType.DMA((U,)),
            pltpu.SemaphoreType.DMA((NSLOT,)),
            pltpu.SemaphoreType.DMA((NSLOT,)),
            pltpu.SemaphoreType.DMA((NSLOT,)),
            pltpu.SemaphoreType.DMA((NSLOT,)),
            pltpu.SemaphoreType.DMA((4,)),
            pltpu.SemaphoreType.DMA((U + 3,)),
        ],
        compiler_params=pltpu.CompilerParams(
            dimension_semantics=("arbitrary",),
            vmem_limit_bytes=100 * 1024 * 1024,
            disable_bounds_checks=True,
            disable_semaphore_checks=True),
        name="fused_attn_moe",
    )(A_x.reshape(S, D), jnp.swapaxes(A_k_cache, 2, 3), jnp.swapaxes(A_v_cache, 2, 3), A_wq, A_wo, B_w_r,
      B_w_gate, B_w_up, B_w_down)
    return out.reshape(B, S, D)
```
